```python
import jax
import jax.numpy as jnp

def _softmax(x, axis=-1):
    return jax.nn.softmax(x, axis=axis)
def _gelu(x):
    return jax.nn.gelu(x, approximate=True)
def _silu(x):
    return jax.nn.silu(x)
def _sigmoid(x):
    return jax.nn.sigmoid(x)
def _layernorm(x, axis=-1, eps=1e-5):
    m = jnp.mean(x, axis=axis, keepdims=True)
    v = jnp.var(x, axis=axis, keepdims=True)
    return (x - m) / jnp.sqrt(v + eps)
def _scatter_add(tgt, idx, src, axis=0):
    return tgt.at[idx].add(src)
def _segment_sum(src, seg, n):
    return jax.ops.segment_sum(src, seg, n)
class _Rng:
    def __init__(self, key):
        self._k = key
    def _next(self):
        self._k, sub = jax.random.split(self._k)
        return sub
    def normal(self, shape):
        return jax.random.normal(self._next(), shape, dtype=jnp.bfloat16)
    def randint(self, lo, hi, shape):
        return jax.random.randint(self._next(), shape, lo, hi, dtype=jnp.int32)
    def uniform(self, shape, lo=0.0, hi=1.0):
        return jax.random.uniform(self._next(), shape, jnp.bfloat16, lo, hi)
    def permutation(self, n):
        return jax.random.permutation(self._next(), n)


kernel_name = 'interleave_layers__sliding_local_dilated__linear_kernel_hedgehog__prompt'

def setup_inputs():
    _rng = _Rng(jax.random.key(int.from_bytes(__import__("os").urandom(4), "little")))
    _w = (lambda a: (lambda t: t.astype(jnp.bfloat16) if jnp.issubdtype(t.dtype, jnp.floating) else t)(jnp.asarray(a)))
    def _A_setup():
        B, S, D = 1, 2048, 1024
        return {
            "x": _w((lambda *s: _rng.normal(s) * 0.05)(B, S, D)),
            "wqkv": _w((lambda *s: _rng.normal(s) * 0.05)(D, 3 * D)),
            "wo": _w((lambda *s: _rng.normal(s) * 0.05)(D, D)),
        }
    _A_in = _A_setup()

    def _B_setup():
        B, S, D, H = 1, 2048, 1024, 32
        Dh = D // H
        return {
            "x": _w((lambda *s: _rng.normal(s) * 0.05)(B, S, D)),
            "wqkv": _w((lambda *s: _rng.normal(s) * 0.05)(D, 3 * D)),
            "w_phi": _w((lambda *s: _rng.normal(s) * 0.05)(H, Dh, Dh) * (Dh ** -0.5)),
            "wo": _w((lambda *s: _rng.normal(s) * 0.05)(D, D)),
        }
    _B_in = _B_setup()

    return {
        "A_x": _A_in["x"],
        "A_wqkv": _A_in["wqkv"],
        "A_wo": _A_in["wo"],
        "B_x": _B_in["x"],
        "B_wqkv": _B_in["wqkv"],
        "B_w_phi": _B_in["w_phi"],
        "B_wo": _B_in["wo"],
    }

def reference(A_x, A_wqkv, A_wo, B_x, B_wqkv, B_w_phi, B_wo):
    def _A_ref(x, wqkv, wo):
        B, S, D = x.shape
        H = 32; Dh = D // H
        W, dil = 8, 2
        qkv = (lambda x, *d: x.transpose(*d))((x @ wqkv).reshape(B, S, 3, H, Dh), 2, 0, 3, 1, 4)
        q, k, v = qkv[0], qkv[1], qkv[2]
        scale = Dh ** -0.5
        pos = jnp.arange(S)
        off = jnp.arange(W) * dil
        idx = pos[:, None] - off[None, :]
        mask = idx >= 0
        idx_c = jnp.where(mask, idx, 0).reshape(-1)
        kg = k[:, :, idx_c, :].reshape(B, H, S, W, Dh)
        vg = v[:, :, idx_c, :].reshape(B, H, S, W, Dh)
        logits = jnp.einsum("bhsd,bhswd->bhsw", q, kg) * scale
        logits = jnp.where(mask[None, None, :, :], logits, -1e9)
        attn = _softmax(logits, axis=-1)
        o = jnp.einsum("bhsw,bhswd->bhsd", attn, vg)
        return (lambda x, *d: x.transpose(*d))(o, 0, 2, 1, 3).reshape(B, S, D) @ wo

    def _B_ref(x, wqkv, w_phi, wo):
        B, S, D = x.shape
        H = 32; Dh = D // H
        qkv = (lambda x, *d: x.transpose(*d))((x @ wqkv).reshape(B, S, 3, H, Dh), 2, 0, 3, 1, 4)
        q, k, v = qkv[0], qkv[1], qkv[2]
        pq = jnp.einsum("bhsd,hdf->bhsf", q, w_phi)
        pk = jnp.einsum("bhsd,hdf->bhsf", k, w_phi)
        phi_q = jnp.concatenate([_softmax(pq, axis=-1), _softmax(-pq, axis=-1)], axis=-1)
        phi_k = jnp.concatenate([_softmax(pk, axis=-1), _softmax(-pk, axis=-1)], axis=-1)
        kv = jnp.einsum("bhsf,bhsd->bhfd", phi_k, v)
        z  = jnp.einsum("bhsf->bhf", phi_k)
        num = jnp.einsum("bhqf,bhfd->bhqd", phi_q, kv)
        den = jnp.einsum("bhqf,bhf->bhq", phi_q, z)[..., None] + 1e-6
        o = num / den
        return (lambda x, *d: x.transpose(*d))(o, 0, 2, 1, 3).reshape(B, S, D) @ wo

    x = A_x
    x = x + _A_ref(_layernorm(x, axis=-1), A_wqkv, A_wo)
    x = x + _B_ref(_layernorm(x, axis=-1), B_wqkv, B_w_phi, B_wo)
    x = x + _A_ref(_layernorm(x, axis=-1), A_wqkv, A_wo)
    x = x + _B_ref(_layernorm(x, axis=-1), B_wqkv, B_w_phi, B_wo)
    return x
```

```python
import jax
import jax.numpy as jnp
from jax import lax
import jax.experimental.pallas as pl
import jax.experimental.pallas.tpu as pltpu

S, D, H, DH, W = 2048, 1024, 32, 32, 8
NT = 512
NB = NT // 128
T = S // NT
LOG2E = 1.4426950408889634
F32, BF16, U32 = jnp.float32, jnp.bfloat16, jnp.uint32


def _dot(a, b):
    return jnp.dot(a, b, preferred_element_type=F32)


def _dot_nt(a, b):
    return lax.dot_general(a, b, (((1,), (1,)), ((), ())), preferred_element_type=F32)


def _unpack(u):
    lo = pltpu.bitcast(u << 16, F32)
    hi = pltpu.bitcast(u & jnp.uint32(0xFFFF0000), F32)
    return lo, hi


def _ln(x):
    m = jnp.mean(x, axis=0, keepdims=True)
    c = x - m
    v = jnp.mean(c * c, axis=0, keepdims=True)
    return (c * lax.rsqrt(v + 1e-5)).astype(BF16)


def _dual_softmax(p):
    ep = jnp.exp2(p - jnp.max(p, axis=0, keepdims=True))
    en = jnp.exp2(jnp.min(p, axis=0, keepdims=True) - p)
    ep = ep * (1.0 / jnp.sum(ep, axis=0, keepdims=True))
    en = en * (1.0 / jnp.sum(en, axis=0, keepdims=True))
    return jnp.concatenate([ep, en], axis=0).astype(BF16)


def _kernel(x_hbm, awqkv_hbm, awo_hbm, bwqkv_hbm, bwphi_ref, bwo_hbm, o_hbm,
            xio, stage, wos, tb, wa, wao, wb, wbo, xt, xn, k2, v2, ob, kvb, sems):
    def wcopy(src, col, slot, sem):
        return pltpu.make_async_copy(src.at[:, pl.ds(col * D, D)], stage.at[slot], sems.at[sem])

    cx = [pltpu.make_async_copy(x_hbm.at[:, pl.ds(c * 128, 128)], xio.at[c], sems.at[0]) for c in range(8)]
    for c in cx:
        c.start()
    cps = [wcopy(awqkv_hbm, c, i, i + 1) for i, c in enumerate((1, 2, 0))]
    cwo = [pltpu.make_async_copy(awo_hbm.at[:, pl.ds(c * 128, 128)], wos.at[c], sems.at[4]) for c in range(8)]
    cps.append(None)
    srcs = [(bwqkv_hbm, 1), (bwqkv_hbm, 2), (bwqkv_hbm, 0), (bwo_hbm, 0)]
    cps += [wcopy(s, c, i + 3, i + 5) for i, (s, c) in enumerate(srcs)]
    for c in cps[:3] + cwo + cps[4:]:
        c.start()

    for c in cx:
        c.wait()
    xu = xio.bitcast(U32)

    def in_body(m, _):
        lo, hi = _unpack(jnp.concatenate([xu[c, pl.ds(m, 128, stride=8), :].T for c in range(8)], 0))
        for p, val in ((0, lo), (1, hi)):
            col = (p * 8 + m) * 128
            xt[:, pl.ds(col, 128)] = val
            xn[:, pl.ds(col, 128)] = _ln(val)
        return 0
    for m in range(8):
        in_body(m, 0)

    def prep_a(part):
        def body(g, _):
            r = pl.multiple_of(g * 256, 256)
            tu = tb.bitcast(U32)
            for c in range(8):
              tb[c] = stage[part, c * 128:(c + 1) * 128, pl.ds(r, 256)].T
              for e in range(16):
                lo, hi = _unpack(tu[c, pl.ds(e, 8, stride=16), :])
                wa[pl.ds(part * D + r + e * 16, 16), c * 128:(c + 1) * 128] = jnp.concatenate([lo, hi], 0).astype(BF16)
            return 0
        lax.fori_loop(0, 4, body, 0)

    cps[0].wait()
    prep_a(0)
    cps[1].wait()
    prep_a(1)
    cps[2].wait()
    prep_a(2)
    for c in cwo:
        c.wait()
    su = wos.bitcast(U32)
    for g in range(4):
      for c in range(8):
        rows = []
        for e in range(16):
            rows += list(_unpack(su[c, pl.ds(g * 128 + e, 8, stride=16), :]))
        wao[c * 128:(c + 1) * 128, g * 256:(g + 1) * 256] = jnp.concatenate(rows, 0).astype(BF16).T

    cps[4].wait()
    cps[6].wait()
    zero = jnp.zeros((32, 32), F32)
    for g in range(8):
        bd = jnp.concatenate(
            [jnp.concatenate([bwphi_ref[4 * g + i].astype(F32) if i == j else zero for j in range(4)], 1)
             for i in range(4)], 0).T.astype(BF16)
        for part in (0, 2):
            wt = stage[3 + part, :, g * 128:(g + 1) * 128].T
            wb[part * D + g * 128: part * D + (g + 1) * 128, :] = (_dot(bd, wt) * LOG2E).astype(BF16)
    cps[5].wait()
    cps[7].wait()
    for g in range(4):
        wb[D + g * 256: D + (g + 1) * 256, :] = stage[4, :, g * 256:(g + 1) * 256].T
        wbo[g * 256:(g + 1) * 256, :] = stage[6, :, g * 256:(g + 1) * 256].T

    def out_proj(w, cols):
        xnew = xt[:, cols] + _dot(w[...], ob[:, 0:NT])
        xt[:, cols] = xnew
        xn[:, cols] = _ln(xnew)

    def layer_a():
        def kv_body(t, _):
            cols = pl.ds(pl.multiple_of(t * NT, NT), NT)
            base = t * NB + 8 * (t * NB // 8)
            for part, dst in ((0, k2), (1, v2)):
                r = _dot(wa[part * D:(part + 1) * D, :], xn[:, cols])
                for i in range(NB):
                    blk = r[:, i * 128:(i + 1) * 128]
                    dst[base + i + 8] = blk
                    dst[base + i] = pltpu.roll(blk, 1, 1)
            return 0
        lax.fori_loop(0, T, kv_body, 0)

        def q_body(t, _):
            cols = pl.ds(pl.multiple_of(t * NT, NT), NT)
            base = t * NB + 8 * (t * NB // 8)
            m0 = t * NB % 8
            lane0 = lax.broadcasted_iota(jnp.int32, (8, 128), 1) == 0
            for g in range(4):
                q = _dot(wa[2 * D + g * 256: 2 * D + (g + 1) * 256, :], xn[:, cols])
                outs = []
                for i in range(NB):
                    lg = []
                    for w in range(W):
                        acc = None
                        for d in range(DH):
                            pr = (q[d * 8:(d + 1) * 8, i * 128:(i + 1) * 128]
                                  * k2[base + i + 8 - w, g * 256 + d * 8: g * 256 + (d + 1) * 8, :])
                            acc = pr if acc is None else acc + pr
                        acc = acc * (DH ** -0.5 * LOG2E)
                        if w > i:
                            acc = jnp.where(jnp.logical_and(lane0, m0 + i < w), -1e9 * LOG2E, acc)
                        lg.append(acc)
                    mx = lg[0]
                    for w in range(1, W):
                        mx = jnp.maximum(mx, lg[w])
                    es = [jnp.exp2(l - mx) for l in lg]
                    tot = es[0]
                    for w in range(1, W):
                        tot = tot + es[w]
                    inv = 1.0 / tot
                    ps = [e * inv for e in es]
                    rows = []
                    for d in range(DH):
                        acc = None
                        for w in range(W):
                            pr = ps[w] * v2[base + i + 8 - w, g * 256 + d * 8: g * 256 + (d + 1) * 8, :]
                            acc = pr if acc is None else acc + pr
                        rows.append(acc)
                    ob[g * 256:(g + 1) * 256, i * 128:(i + 1) * 128] = jnp.concatenate(rows, 0).astype(BF16)
            out_proj(wao, cols)
            return 0
        lax.fori_loop(0, T, q_body, 0)

    def layer_b():
        kvb[...] = jnp.zeros(kvb.shape, F32)

        def kv_body(t, _):
            cols = pl.ds(pl.multiple_of(t * NT, NT), NT)
            ones = jnp.ones((16, NT), BF16)
            for g in range(4):
                k = _dot(wb[g * 256:(g + 1) * 256, :], xn[:, cols])
                v = _dot(wb[D + g * 256: D + (g + 1) * 256, :], xn[:, cols]).astype(BF16)
                for i in range(4):
                    phi = jnp.concatenate([_dual_softmax(k[i * 64:i * 64 + 32]),
                                           _dual_softmax(k[i * 64 + 32:i * 64 + 64])], 0)
                    lhs = jnp.concatenate([v[i * 64:(i + 1) * 64], ones], 0)
                    kvb[g * 4 + i] += _dot_nt(lhs, phi)
            return 0
        lax.fori_loop(0, T, kv_body, 0)
        r = lax.broadcasted_iota(jnp.int32, (80, 128), 0)
        c = lax.broadcasted_iota(jnp.int32, (80, 128), 1)
        keep = jnp.where(r < 64, r // 32, (r - 64) // 8) == c // 64
        for i in range(16):
            kvb[i] = jnp.where(keep, kvb[i], 0.0)

        def q_body(t, _):
            cols = pl.ds(pl.multiple_of(t * NT, NT), NT)
            for g in range(4):
                q = _dot(wb[2 * D + g * 256: 2 * D + (g + 1) * 256, :], xn[:, cols])
                for i in range(4):
                    phi = jnp.concatenate([_dual_softmax(q[i * 64:i * 64 + 32]),
                                           _dual_softmax(q[i * 64 + 32:i * 64 + 64])], 0)
                    nd = _dot(kvb[g * 4 + i].astype(BF16), phi)
                    rows = []
                    for hh in range(2):
                        inv = 1.0 / (nd[64 + hh * 8:72 + hh * 8] + 1e-6)
                        rows += [nd[hh * 32 + j * 8: hh * 32 + (j + 1) * 8] * inv for j in range(4)]
                    ob[g * 256 + i * 64: g * 256 + (i + 1) * 64, 0:NT] = jnp.concatenate(rows, 0).astype(BF16)
            out_proj(wbo, cols)
            return 0
        lax.fori_loop(0, T, q_body, 0)

    def pair(_, c):
        layer_a()
        layer_b()
        return c
    lax.fori_loop(0, 2, pair, 0)

    def out_body(m, _):
        both = []
        for p in range(2):
            col = (p * 8 + m) * 128
            both.append(pltpu.bitcast(xt[:, pl.ds(col, 128)].astype(BF16).astype(F32), U32))
        u = (both[0] >> 16) | both[1]
        for c in range(8):
            xu[c, pl.ds(m, 128, stride=8), :] = u[c * 128:(c + 1) * 128].T
        return 0
    for m in range(8):
        out_body(m, 0)
    co = [pltpu.make_async_copy(xio.at[c], o_hbm.at[:, pl.ds(c * 128, 128)], sems.at[9]) for c in range(8)]
    for c in co:
        c.start()
    for c in co:
        c.wait()


@jax.jit
def pallas_interleave_layers__sliding_local_dilated__linear_kernel_hedgehog__prompt_kernel(
    A_x, A_wqkv, A_wo, B_x, B_wqkv, B_w_phi, B_wo,
):
    hbm = pl.BlockSpec(memory_space=pl.ANY)
    out = pl.pallas_call(
        _kernel,
        out_shape=jax.ShapeDtypeStruct((S, D), BF16),
        in_specs=[hbm, hbm, hbm, hbm, pl.BlockSpec(memory_space=pltpu.VMEM), hbm],
        out_specs=hbm,
        scratch_shapes=[
            pltpu.VMEM((8, S, 128), BF16),
            pltpu.VMEM((7, D, D), BF16),
            pltpu.VMEM((8, D, 128), BF16),
            pltpu.VMEM((8, 256, 128), BF16),
            pltpu.VMEM((3 * D, D), BF16),
            pltpu.VMEM((D, D), BF16),
            pltpu.VMEM((3 * D, D), BF16),
            pltpu.VMEM((D, D), BF16),
            pltpu.VMEM((D, S), F32),
            pltpu.VMEM((D, S), BF16),
            pltpu.VMEM((32, D, 128), F32),
            pltpu.VMEM((32, D, 128), F32),
            pltpu.VMEM((D, D), BF16),
            pltpu.VMEM((16, 80, 128), F32),
            pltpu.SemaphoreType.DMA((10,)),
        ],
        compiler_params=pltpu.CompilerParams(vmem_limit_bytes=120 * 1024 * 1024),
    )(A_x.reshape(S, D), A_wqkv, A_wo, B_wqkv, B_w_phi, B_wo)
    return out.reshape(1, S, D)
```

```python
import jax
import jax.numpy as jnp
from jax import lax
import jax.experimental.pallas as pl
import jax.experimental.pallas.tpu as pltpu

S, D, H, DH, W = 2048, 1024, 32, 32, 8
NT = 512
NB = NT // 128
T = S // NT
LOG2E = 1.4426950408889634
F32, BF16, U32 = jnp.float32, jnp.bfloat16, jnp.uint32


def _dot(a, b):
    return jnp.dot(a, b, preferred_element_type=F32)


def _dot_nt(a, b):
    return lax.dot_general(a, b, (((1,), (1,)), ((), ())), preferred_element_type=F32)


def _rcp(x):
    return pl.reciprocal(x, approx=True)


def _unpack(u):
    lo = pltpu.bitcast(u << 16, F32)
    hi = pltpu.bitcast(u & jnp.uint32(0xFFFF0000), F32)
    return lo, hi


def _ln(x):
    m = jnp.mean(x, axis=0, keepdims=True)
    c = x - m
    v = jnp.mean(c * c, axis=0, keepdims=True)
    return (c * lax.rsqrt(v + 1e-5)).astype(BF16)


def _dual_softmax(p):
    ep = jnp.exp2(p - jnp.max(p, axis=0, keepdims=True))
    en = jnp.exp2(jnp.min(p, axis=0, keepdims=True) - p)
    ep = ep * _rcp(jnp.sum(ep, axis=0, keepdims=True))
    en = en * _rcp(jnp.sum(en, axis=0, keepdims=True))
    return jnp.concatenate([ep, en], axis=0).astype(BF16)


def _kernel(x_hbm, awqkv_hbm, awo_hbm, bwqkv_hbm, bwphi_ref, bwo_hbm, o_hbm,
            xio, stage, wos, tb, wa, wao, wb, wbo, xt, xn, k2, v2, ob, kvb, sems):
    def wcopy(src, col, slot, sem):
        return pltpu.make_async_copy(src.at[:, pl.ds(col * D, D)], stage.at[slot], sems.at[sem])

    cx = [pltpu.make_async_copy(x_hbm.at[:, pl.ds(c * 128, 128)], xio.at[c], sems.at[9 + c]) for c in range(8)]
    for c in cx:
        c.start()
    cps = [wcopy(awqkv_hbm, c, i, i + 1) for i, c in enumerate((1, 2, 0))]
    cwo = [pltpu.make_async_copy(awo_hbm.at[pl.ds(g * 256, 256), pl.ds(c * 128, 128)], wos.at[c * 4 + g], sems.at[4])
           for c in range(8) for g in range(4)]
    cps.append(None)
    srcs = [(bwqkv_hbm, 1), (bwqkv_hbm, 2), (bwqkv_hbm, 0), (bwo_hbm, 0)]
    cps += [wcopy(s, c, i + 3, i + 5) for i, (s, c) in enumerate(srcs)]
    for c in cps[:2]:
        c.start()

    xu = xio.bitcast(U32)

    def in_body(c, _):
        pltpu.make_async_copy(xio.at[0], xio.at[0], sems.at[9 + c]).wait()

        @pl.when(c == 5)
        def _():
            for cp in [cps[2]] + cwo:
                cp.start()
        rows = pl.ds(pl.multiple_of(c * 128, 128), 128)
        for m in range(8):
            lo, hi = _unpack(xu[c, pl.ds(m, 128, stride=8), :].T)
            xt[rows, m * 128:(m + 1) * 128] = lo
            xt[rows, (8 + m) * 128:(9 + m) * 128] = hi
    with jax.named_scope("loop_in"):
        lax.fori_loop(0, 8, in_body, None)
    for cp in cps[4:]:
        cp.start()

    def ln_body(b, _):
        cols = pl.ds(pl.multiple_of(b * 256, 256), 256)
        xn[:, cols] = _ln(xt[:, cols])
    with jax.named_scope("loop_ln"):
        lax.fori_loop(0, S // 256, ln_body, None)

    def prep_a(part, g):
        r = pl.multiple_of(g * 256, 256)
        tu = tb.bitcast(U32)
        for c in range(8):
            tb[c] = stage[part, c * 128:(c + 1) * 128, pl.ds(r, 256)].T
            for e in range(16):
                lo, hi = _unpack(tu[c, pl.ds(e, 8, stride=16), :])
                wa[pl.ds(part * D + r + e * 16, 16), c * 128:(c + 1) * 128] = (
                    jnp.concatenate([lo, hi], 0).astype(BF16))

    def prep_rest(g):
        r = pl.multiple_of(g * 256, 256)
        prep_a(2, g)
        su = wos.bitcast(U32)
        for c in range(8):
            rows = []
            for e in range(16):
                rows += list(_unpack(su[c * 4 + g, pl.ds(e, 8, stride=16), :]))
            wao[c * 128:(c + 1) * 128, pl.ds(r, 256)] = jnp.concatenate(rows, 0).astype(BF16).T

    def prep_b(g):
        r = pl.multiple_of(g * 256, 256)
        zero = jnp.zeros((32, 32), F32)
        for gg in range(2):
            bd = jnp.concatenate(
                [jnp.concatenate([bwphi_ref[8 * g + 4 * gg + i].astype(F32) if i == j else zero
                                  for j in range(4)], 1) for i in range(4)], 0).T.astype(BF16)
            rr = pl.multiple_of(r + gg * 128, 128)
            for part in (0, 2):
                wt = stage[3 + part, :, pl.ds(rr, 128)].T
                wb[pl.ds(part * D + rr, 128), :] = (_dot(bd, wt) * LOG2E).astype(BF16)
        wb[pl.ds(D + r, 256), :] = stage[4, :, pl.ds(r, 256)].T
        wbo[pl.ds(r, 256), :] = stage[6, :, pl.ds(r, 256)].T

    for part in range(2):
        cps[part].wait()
        with jax.named_scope("loop_pa"):
            lax.fori_loop(0, 4, lambda g, c: prep_a(part, g), None)
    for c in [cps[2]] + cwo:
        c.wait()
    with jax.named_scope("loop_pr"):
        lax.fori_loop(0, 4, lambda g, c: prep_rest(g), None)

    def ln_tile(src, dst):
        xn[:, pl.ds(pl.multiple_of(dst * NT, NT), NT)] = _ln(xt[:, pl.ds(pl.multiple_of(src * NT, NT), NT)])

    def out_proj(w, t, part):
        ln_tile(jnp.maximum(t - 1, 0), jnp.where(t == 0, T, t - 1))
        cols = pl.ds(pl.multiple_of(t * NT, NT), NT)
        xnew = part + _dot(w[:, 512:], ob[512:, 0:NT])
        xt[:, cols] = xnew

    def layer_a(it):
        def kv_body(t, _):
            cols = pl.ds(pl.multiple_of(jnp.int32(t) * NT, NT), NT)
            base = t * NB + 8 * (t * NB // 8)
            for part, dst in ((0, k2), (1, v2)):
                r = _dot(wa[part * D:(part + 1) * D, :], xn[:, cols])
                for i in range(NB):
                    blk = r[:, i * 128:(i + 1) * 128]
                    dst[base + i + 8] = blk
                    dst[base + i] = pltpu.roll(blk, 1, 1)
            return 0
        with jax.named_scope("loop137"):
            xn[:, S - NT:S] = _ln(xt[:, S - NT:S])
            kv_body(0, 0)
            lax.fori_loop(1, T, kv_body, 0)

        @pl.when(it == 0)
        def _():
            for c in cps[4:]:
                c.wait()

        def q_body(t, _):
            cols = pl.ds(pl.multiple_of(jnp.int32(t) * NT, NT), NT)
            base = t * NB + 8 * (t * NB // 8)
            m0 = t * NB % 8
            lane0 = lax.broadcasted_iota(jnp.int32, (8, 128), 1) == 0
            qd = lambda g: _dot(wa[2 * D + g * 256: 2 * D + (g + 1) * 256, :], xn[:, cols])
            nxt = qd(0)
            for g in range(4):
                q = nxt
                if g < 3:
                    nxt = qd(g + 1)
                else:
                    nxt = xt[:, cols] + _dot(wao[:, 0:512], ob[0:512, 0:NT])
                outs = []
                for i in range(NB):
                    lg = []
                    for w in range(W):
                        acc = None
                        for d in range(DH):
                            pr = (q[d * 8:(d + 1) * 8, i * 128:(i + 1) * 128]
                                  * k2[base + i + 8 - w, g * 256 + d * 8: g * 256 + (d + 1) * 8, :])
                            acc = pr if acc is None else acc + pr
                        acc = acc * (DH ** -0.5 * LOG2E)
                        if w > i:
                            acc = jnp.where(jnp.logical_and(lane0, m0 + i < w), -1e9 * LOG2E, acc)
                        lg.append(acc)
                    mx = lg[0]
                    for w in range(1, W):
                        mx = jnp.maximum(mx, lg[w])
                    es = [jnp.exp2(l - mx) for l in lg]
                    tot = es[0]
                    for w in range(1, W):
                        tot = tot + es[w]
                    inv = _rcp(tot)
                    ps = [e * inv for e in es]
                    rows = []
                    for d in range(DH):
                        acc = None
                        for w in range(W):
                            pr = ps[w] * v2[base + i + 8 - w, g * 256 + d * 8: g * 256 + (d + 1) * 8, :]
                            acc = pr if acc is None else acc + pr
                        rows.append(acc)
                    ob[g * 256:(g + 1) * 256, i * 128:(i + 1) * 128] = jnp.concatenate(rows, 0).astype(BF16)
            prep_b(t)
            out_proj(wao, t, nxt)
            return 0
        with jax.named_scope("loop178"):
            lax.fori_loop(0, T, q_body, 0)

    def layer_b():
        kvb[...] = jnp.zeros(kvb.shape, F32)

        def kv_body(t, _):
            cols = pl.ds(pl.multiple_of(jnp.int32(t) * NT, NT), NT)
            ones = jnp.ones((16, NT), BF16)
            kd = lambda g: _dot(wb[g * 256:(g + 1) * 256, :], xn[:, cols])
            nxt = kd(0)
            for g in range(4):
                k = nxt
                v = _dot(wb[D + g * 256: D + (g + 1) * 256, :], xn[:, cols]).astype(BF16)
                if g < 3:
                    nxt = kd(g + 1)
                for i in range(4):
                    phi = jnp.concatenate([_dual_softmax(k[i * 64:i * 64 + 32]),
                                           _dual_softmax(k[i * 64 + 32:i * 64 + 64])], 0)
                    lhs = jnp.concatenate([v[i * 64:(i + 1) * 64], ones], 0)
                    kvb[g * 4 + i] += _dot_nt(lhs, phi)
            return 0
        with jax.named_scope("loop195"):
            xn[:, S - NT:S] = _ln(xt[:, S - NT:S])
            kv_body(0, 0)
            lax.fori_loop(1, T, kv_body, 0)
        r = lax.broadcasted_iota(jnp.int32, (80, 128), 0)
        c = lax.broadcasted_iota(jnp.int32, (80, 128), 1)
        keep = jnp.where(r < 64, r // 32, (r - 64) // 8) == c // 64
        for i in range(16):
            kvb[i] = jnp.where(keep, kvb[i], 0.0)

        def q_body(t, _):
            cols = pl.ds(pl.multiple_of(t * NT, NT), NT)
            qd = lambda g: _dot(wb[2 * D + g * 256: 2 * D + (g + 1) * 256, :], xn[:, cols])
            nxt = qd(0)
            for g in range(4):
                q = nxt
                if g < 3:
                    nxt = qd(g + 1)
                else:
                    nxt = xt[:, cols] + _dot(wbo[:, 0:512], ob[0:512, 0:NT])
                for i in range(4):
                    phi = jnp.concatenate([_dual_softmax(q[i * 64:i * 64 + 32]),
                                           _dual_softmax(q[i * 64 + 32:i * 64 + 64])], 0)
                    nd = _dot(kvb[g * 4 + i].astype(BF16), phi)
                    rows = []
                    for hh in range(2):
                        inv = _rcp(nd[64 + hh * 8:72 + hh * 8] + 1e-6)
                        rows += [nd[hh * 32 + j * 8: hh * 32 + (j + 1) * 8] * inv for j in range(4)]
                    ob[g * 256 + i * 64: g * 256 + (i + 1) * 64, 0:NT] = jnp.concatenate(rows, 0).astype(BF16)
            out_proj(wbo, t, nxt)
            return 0
        with jax.named_scope("loop217"):
            lax.fori_loop(0, T, q_body, 0)

    def pair(it, c):
        layer_a(it)
        layer_b()
        return c
    lax.fori_loop(0, 2, pair, 0)

    co = [pltpu.make_async_copy(xio.at[c], o_hbm.at[:, pl.ds(c * 128, 128)], sems.at[0]) for c in range(8)]

    def out_body(c, _):
        rows = pl.ds(pl.multiple_of(c * 128, 128), 128)
        for m in range(8):
            lo, hi = [pltpu.bitcast(xt[rows, b * 128:(b + 1) * 128].astype(BF16).astype(F32), U32)
                      for b in (m, 8 + m)]
            xu[c, pl.ds(m, 128, stride=8), :] = ((lo >> 16) | hi).T
        pltpu.make_async_copy(xio.at[c], o_hbm.at[:, pl.ds(pl.multiple_of(c * 128, 128), 128)], sems.at[0]).start()
    with jax.named_scope("loop_out"):
        lax.fori_loop(0, 8, out_body, None)
    for c in co:
        c.wait()


@jax.jit
def pallas_interleave_layers__sliding_local_dilated__linear_kernel_hedgehog__prompt_kernel(
    A_x, A_wqkv, A_wo, B_x, B_wqkv, B_w_phi, B_wo,
):
    hbm = pl.BlockSpec(memory_space=pl.ANY)
    out = pl.pallas_call(
        _kernel,
        out_shape=jax.ShapeDtypeStruct((S, D), BF16),
        in_specs=[hbm, hbm, hbm, hbm, pl.BlockSpec(memory_space=pltpu.VMEM), hbm],
        out_specs=hbm,
        scratch_shapes=[
            pltpu.VMEM((8, S, 128), BF16),
            pltpu.VMEM((7, D, D), BF16),
            pltpu.VMEM((32, 256, 128), BF16),
            pltpu.VMEM((8, 256, 128), BF16),
            pltpu.VMEM((3 * D, D), BF16),
            pltpu.VMEM((D, D), BF16),
            pltpu.VMEM((3 * D, D), BF16),
            pltpu.VMEM((D, D), BF16),
            pltpu.VMEM((D, S), F32),
            pltpu.VMEM((D, S + NT), BF16),
            pltpu.VMEM((32, D, 128), F32),
            pltpu.VMEM((32, D, 128), F32),
            pltpu.VMEM((D, D), BF16),
            pltpu.VMEM((16, 80, 128), F32),
            pltpu.SemaphoreType.DMA((17,)),
        ],
        compiler_params=pltpu.CompilerParams(vmem_limit_bytes=120 * 1024 * 1024),
    )(A_x.reshape(S, D), A_wqkv, A_wo, B_wqkv, B_w_phi, B_wo)
    return out.reshape(1, S, D)
```

```python
import jax
import jax.numpy as jnp
from jax import lax
import jax.experimental.pallas as pl
import jax.experimental.pallas.tpu as pltpu

S, D, H, DH, W = 2048, 1024, 32, 32, 8
NT = 512
NB = NT // 128
T = S // NT
LOG2E = 1.4426950408889634
F32, BF16, U32 = jnp.float32, jnp.bfloat16, jnp.uint32


def _dot(a, b):
    return jnp.dot(a, b, preferred_element_type=F32)


def _dot_nt(a, b):
    return lax.dot_general(a, b, (((1,), (1,)), ((), ())), preferred_element_type=F32)


def _rcp(x):
    return pl.reciprocal(x, approx=True)


def _unpack(u):
    lo = pltpu.bitcast(u << 16, F32)
    hi = pltpu.bitcast(u & jnp.uint32(0xFFFF0000), F32)
    return lo, hi


def _ln(x):
    m = jnp.mean(x, axis=0, keepdims=True)
    c = x - m
    v = jnp.mean(c * c, axis=0, keepdims=True)
    return c * lax.rsqrt(v + 1e-5)


def _rhs7(b11, b12, b21, b22):
    return [v.astype(BF16) for v in (b11 + b22, b11, b12 - b22, b21 - b11, b22, b11 + b12, b21 + b22)]


def _lhs7(a11, a12, a21, a22):
    return [v.astype(BF16) for v in (a11 + a22, a21 + a22, a11, a22, a11 + a12, a21 - a11, a12 - a22)]


def _dual_softmax(p):
    ep = jnp.exp2(p - jnp.max(p, axis=0, keepdims=True))
    en = jnp.exp2(jnp.min(p, axis=0, keepdims=True) - p)
    ep = ep * _rcp(jnp.sum(ep, axis=0, keepdims=True))
    en = en * _rcp(jnp.sum(en, axis=0, keepdims=True))
    return jnp.concatenate([ep, en], axis=0).astype(BF16)


def _kernel(x_hbm, awqkv_hbm, awo_hbm, bwqkv_hbm, bwphi_ref, bwo_hbm, o_hbm,
            xio, stage, wos, tb, ws, xt, xs, k2, v2, os_, kvb, sems):
    def wcopy(src, col, slot, sem):
        return pltpu.make_async_copy(src.at[:, pl.ds(col * D, D)], stage.at[slot], sems.at[sem])

    cx = [pltpu.make_async_copy(x_hbm.at[:, pl.ds(c * 128, 128)], xio.at[c], sems.at[9 + c]) for c in range(8)]
    for c in cx:
        c.start()
    cps = [wcopy(awqkv_hbm, c, i, i + 1) for i, c in enumerate((1, 2, 0))]
    cwo = [pltpu.make_async_copy(awo_hbm.at[pl.ds(g * 256, 256), pl.ds(c * 128, 128)], wos.at[c * 4 + g], sems.at[4])
           for c in range(8) for g in range(4)]
    cps.append(None)
    srcs = [(bwqkv_hbm, 1), (bwqkv_hbm, 2), (bwqkv_hbm, 0), (bwo_hbm, 0)]
    cps += [wcopy(s, c, i + 3, i + 5) for i, (s, c) in enumerate(srcs)]
    for c in cps[:2]:
        c.start()

    xu = xio.bitcast(U32)

    def in_body(c, _):
        pltpu.make_async_copy(xio.at[0], xio.at[0], sems.at[9 + c]).wait()

        @pl.when(c == 5)
        def _():
            for cp in [cps[2]] + cwo:
                cp.start()
        rows = pl.ds(pl.multiple_of(c * 128, 128), 128)
        for m in range(8):
            lo, hi = _unpack(xu[c, pl.ds(m, 128, stride=8), :].T)
            xt[rows, m * 128:(m + 1) * 128] = lo
            xt[rows, (8 + m) * 128:(9 + m) * 128] = hi
    with jax.named_scope("loop_in"):
        lax.fori_loop(0, 8, in_body, None)
    for cp in cps[4:]:
        cp.start()

    def ln_tile(src, dst):
        y = _ln(xt[:, pl.ds(pl.multiple_of(src * NT, NT), NT)])
        for i, v in enumerate(_rhs7(y[:512, :256], y[:512, 256:], y[512:, :256], y[512:, 256:])):
            xs[dst, i] = v
    with jax.named_scope("loop_ln"):
        lax.fori_loop(0, T, lambda t, c: ln_tile(t, t), None)

    def emit(mat, mc, r0, c0, *quads):
        for i, v in enumerate(_lhs7(*quads)):
            ws[mat * 2 + mc, i, r0:r0 + v.shape[0], c0:c0 + v.shape[1]] = v

    def prep_a(part, mc):
        tu = tb.bitcast(U32)
        for c in range(4):
            quads = []
            for j, (g, cc) in enumerate(((mc, c), (mc, c + 4), (mc + 2, c), (mc + 2, c + 4))):
                tb[j] = stage[part, cc * 128:(cc + 1) * 128, pl.ds(pl.multiple_of(g * 256, 256), 256)].T
                rows = []
                for e in range(16):
                    rows += list(_unpack(tu[j, pl.ds(e, 8, stride=16), :]))
                quads.append(jnp.concatenate(rows, 0))
            emit(part, mc, 0, c * 128, *quads)

    def prep_rest(mc):
        prep_a(2, mc)
        su = wos.bitcast(U32)
        for c in range(2):
            for gk in range(2):
                quads = []
                for cc, g in ((2 * mc + c, gk), (2 * mc + c, gk + 2), (2 * mc + c + 4, gk), (2 * mc + c + 4, gk + 2)):
                    rows = []
                    for e in range(16):
                        rows += list(_unpack(su[cc * 4 + g, pl.ds(e, 8, stride=16), :]))
                    quads.append(jnp.concatenate(rows, 0).T)
                emit(3, mc, c * 128, gk * 256, *quads)

    def prep_plain(slot, mat, mc):
        for c in range(4):
            quads = [stage[slot, cc * 128:(cc + 1) * 128, pl.ds(pl.multiple_of(g * 256, 256), 256)].T.astype(F32)
                     for g, cc in ((mc, c), (mc, c + 4), (mc + 2, c), (mc + 2, c + 4))]
            emit(mat, mc, 0, c * 128, *quads)

    def prep_fold(part, mc):
        zero = jnp.zeros((32, 32), F32)
        for gg in range(2):
            r = []
            for g in (mc, mc + 2):
                bd = jnp.concatenate(
                    [jnp.concatenate([bwphi_ref[8 * g + 4 * gg + i].astype(F32) if i == j else zero
                                      for j in range(4)], 1) for i in range(4)], 0).T.astype(BF16)
                wt = stage[3 + part, :, pl.ds(pl.multiple_of(g * 256 + gg * 128, 128), 128)].T
                r.append(_dot(bd, wt) * LOG2E)
            emit(4 + part, mc, gg * 128, 0, r[0][:, :512], r[0][:, 512:], r[1][:, :512], r[1][:, 512:])

    for part in range(2):
        cps[part].wait()
        with jax.named_scope("loop_pa"):
            lax.fori_loop(0, 2, lambda g, c: prep_a(part, g), None)
    for c in [cps[2]] + cwo:
        c.wait()
    with jax.named_scope("loop_pr"):
        lax.fori_loop(0, 2, lambda g, c: prep_rest(g), None)

    def sdot(mat, mc, rhs, k0=0, k1=512):
        p = [_dot(ws[mat * 2 + mc, i, :, k0:k1], rhs(i)[k0:k1, :]) for i in range(7)]
        return (jnp.concatenate([p[0] + p[3] - p[4] + p[6], p[2] + p[4]], 1),
                jnp.concatenate([p[1] + p[3], p[0] - p[1] + p[2] + p[5]], 1))

    def xdot(mat, mc, t):
        return sdot(mat, mc, lambda i: xs.at[t, i])

    def wo_part(mat, half, cols):
        for mc in range(2):
            for g, r in zip((mc, mc + 2), sdot(mat, mc, lambda i: os_.at[i], half * 256, half * 256 + 256)):
                xt[g * 256:(g + 1) * 256, cols] += r

    def emit_o(half, r0, c0, *quads):
        for i, v in enumerate(_rhs7(*quads)):
            os_[i, half * 256 + r0:half * 256 + r0 + v.shape[0], c0:c0 + v.shape[1]] = v

    def layer_a(it):
        def kv_body(t, _):
            cols = pl.ds(pl.multiple_of(jnp.int32(t) * NT, NT), NT)
            base = t * NB + 8 * (t * NB // 8)
            for part, dst in ((0, k2), (1, v2)):
                for mc in range(2):
                    for g, r in zip((mc, mc + 2), xdot(part, mc, t)):
                        for i in range(NB):
                            blk = r[:, i * 128:(i + 1) * 128]
                            dst[base + i + 8, g * 256:(g + 1) * 256] = blk
                            dst[base + i, g * 256:(g + 1) * 256] = pltpu.roll(blk, 1, 1)
            return 0
        with jax.named_scope("loop137"):
            ln_tile(T - 1, T - 1)
            kv_body(0, 0)
            lax.fori_loop(1, T, kv_body, 0)

        @pl.when(it == 0)
        def _():
            for c in cps[4:]:
                c.wait()

        def q_body(t, _):
            cols = pl.ds(pl.multiple_of(jnp.int32(t) * NT, NT), NT)
            base = t * NB + 8 * (t * NB // 8)
            m0 = t * NB % 8
            lane0 = lax.broadcasted_iota(jnp.int32, (8, 128), 1) == 0
            qs = [xdot(2, 0, t), xdot(2, 1, t)]
            for g in (0, 2, 1, 3):
                q = qs[g % 2][g // 2]
                if g == 1:
                    wo_part(3, 0, cols)
                if g < 2:
                    outs = []
                for i in range(NB):
                    lg = []
                    for w in range(W):
                        acc = None
                        for d in range(DH):
                            pr = (q[d * 8:(d + 1) * 8, i * 128:(i + 1) * 128]
                                  * k2[base + i + 8 - w, g * 256 + d * 8: g * 256 + (d + 1) * 8, :])
                            acc = pr if acc is None else acc + pr
                        acc = acc * (DH ** -0.5 * LOG2E)
                        if w > i:
                            acc = jnp.where(jnp.logical_and(lane0, m0 + i < w), -1e9 * LOG2E, acc)
                        lg.append(acc)
                    mx = lg[0]
                    for w in range(1, W):
                        mx = jnp.maximum(mx, lg[w])
                    es = [jnp.exp2(l - mx) for l in lg]
                    tot = es[0]
                    for w in range(1, W):
                        tot = tot + es[w]
                    inv = _rcp(tot)
                    ps = [e * inv for e in es]
                    rows = []
                    for d in range(DH):
                        acc = None
                        for w in range(W):
                            pr = ps[w] * v2[base + i + 8 - w, g * 256 + d * 8: g * 256 + (d + 1) * 8, :]
                            acc = pr if acc is None else acc + pr
                        rows.append(acc)
                    outs.append(jnp.concatenate(rows, 0))
                if g >= 2:
                    for i in range(2):
                        emit_o(g - 2, 0, i * 128, outs[i], outs[i + 2], outs[4 + i], outs[6 + i])
            prep_fold(2 * (t // 2), t % 2)
            prep_plain(4 + 2 * (t // 2), 5 + 2 * (t // 2), t % 2)
            wo_part(3, 1, cols)
            ln_tile(t, t)
            return 0
        with jax.named_scope("loop178"):
            lax.fori_loop(0, T, q_body, 0)

    def layer_b():
        kvb[...] = jnp.zeros(kvb.shape, F32)

        def kv_body(t, _):
            cols = pl.ds(pl.multiple_of(jnp.int32(t) * NT, NT), NT)
            ones = jnp.ones((16, NT), BF16)
            ks = [xdot(4, mc, t) for mc in range(2)]
            vs = [xdot(5, mc, t) for mc in range(2)]
            for g in (0, 2, 1, 3):
                k = ks[g % 2][g // 2]
                v = vs[g % 2][g // 2].astype(BF16)
                for i in range(4):
                    phi = jnp.concatenate([_dual_softmax(k[i * 64:i * 64 + 32]),
                                           _dual_softmax(k[i * 64 + 32:i * 64 + 64])], 0)
                    lhs = jnp.concatenate([v[i * 64:(i + 1) * 64], ones], 0)
                    kvb[g * 4 + i] += _dot_nt(lhs, phi)
            return 0
        with jax.named_scope("loop195"):
            ln_tile(T - 1, T - 1)
            kv_body(0, 0)
            lax.fori_loop(1, T, kv_body, 0)
        r = lax.broadcasted_iota(jnp.int32, (80, 128), 0)
        c = lax.broadcasted_iota(jnp.int32, (80, 128), 1)
        keep = jnp.where(r < 64, r // 32, (r - 64) // 8) == c // 64
        for i in range(16):
            kvb[i] = jnp.where(keep, kvb[i], 0.0)

        def q_body(t, _):
            cols = pl.ds(pl.multiple_of(t * NT, NT), NT)
            qs = [xdot(6, 0, t), xdot(6, 1, t)]
            for g in (0, 2, 1, 3):
                q = qs[g % 2][g // 2]
                if g == 1:
                    wo_part(7, 0, cols)
                if g < 2:
                    outs = []
                for i in range(4):
                    phi = jnp.concatenate([_dual_softmax(q[i * 64:i * 64 + 32]),
                                           _dual_softmax(q[i * 64 + 32:i * 64 + 64])], 0)
                    nd = _dot(kvb[g * 4 + i].astype(BF16), phi)
                    rows = []
                    for hh in range(2):
                        inv = _rcp(nd[64 + hh * 8:72 + hh * 8] + 1e-6)
                        rows += [nd[hh * 32 + j * 8: hh * 32 + (j + 1) * 8] * inv for j in range(4)]
                    outs.append(jnp.concatenate(rows, 0))
                    if g >= 2:
                        emit_o(g - 2, i * 64, 0, outs[i][:, :256], outs[i][:, 256:],
                               outs[4 + i][:, :256], outs[4 + i][:, 256:])
            ln_tile(jnp.maximum(t - 1, 0), jnp.where(t == 0, T, t - 1))
            wo_part(7, 1, cols)
            return 0
        with jax.named_scope("loop217"):
            lax.fori_loop(0, T, q_body, 0)

    def pair(it, c):
        layer_a(it)
        layer_b()
        return c
    lax.fori_loop(0, 2, pair, 0)

    co = [pltpu.make_async_copy(xio.at[c], o_hbm.at[:, pl.ds(c * 128, 128)], sems.at[0]) for c in range(8)]

    def out_body(c, _):
        rows = pl.ds(pl.multiple_of(c * 128, 128), 128)
        for m in range(8):
            lo, hi = [pltpu.bitcast(xt[rows, b * 128:(b + 1) * 128].astype(BF16).astype(F32), U32)
                      for b in (m, 8 + m)]
            xu[c, pl.ds(m, 128, stride=8), :] = ((lo >> 16) | hi).T
        pltpu.make_async_copy(xio.at[c], o_hbm.at[:, pl.ds(pl.multiple_of(c * 128, 128), 128)], sems.at[0]).start()
    with jax.named_scope("loop_out"):
        lax.fori_loop(0, 8, out_body, None)
    for c in co:
        c.wait()


@jax.jit
def pallas_interleave_layers__sliding_local_dilated__linear_kernel_hedgehog__prompt_kernel(
    A_x, A_wqkv, A_wo, B_x, B_wqkv, B_w_phi, B_wo,
):
    hbm = pl.BlockSpec(memory_space=pl.ANY)
    out = pl.pallas_call(
        _kernel,
        out_shape=jax.ShapeDtypeStruct((S, D), BF16),
        in_specs=[hbm, hbm, hbm, hbm, pl.BlockSpec(memory_space=pltpu.VMEM), hbm],
        out_specs=hbm,
        scratch_shapes=[
            pltpu.VMEM((8, S, 128), BF16),
            pltpu.VMEM((7, D, D), BF16),
            pltpu.VMEM((32, 256, 128), BF16),
            pltpu.VMEM((4, 256, 128), BF16),
            pltpu.VMEM((16, 7, 256, 512), BF16),
            pltpu.VMEM((D, S), F32),
            pltpu.VMEM((T + 1, 7, 512, 256), BF16),
            pltpu.VMEM((32, D, 128), F32),
            pltpu.VMEM((32, D, 128), F32),
            pltpu.VMEM((7, 512, 256), BF16),
            pltpu.VMEM((16, 80, 128), F32),
            pltpu.SemaphoreType.DMA((17,)),
        ],
        compiler_params=pltpu.CompilerParams(vmem_limit_bytes=126 * 1024 * 1024),
    )(A_x.reshape(S, D), A_wqkv, A_wo, B_wqkv, B_w_phi, B_wo)
    return out.reshape(1, S, D)
```

```python
import jax
import jax.numpy as jnp
from jax import lax
import jax.experimental.pallas as pl
import jax.experimental.pallas.tpu as pltpu

S, D, H, DH, W = 2048, 1024, 32, 32, 8
NT = 512
NB = NT // 128
T = S // NT
LOG2E = 1.4426950408889634
F32, BF16, U32 = jnp.float32, jnp.bfloat16, jnp.uint32


def _dot(a, b):
    return jnp.dot(a, b, preferred_element_type=F32)


def _dot_nt(a, b):
    return lax.dot_general(a, b, (((1,), (1,)), ((), ())), preferred_element_type=F32)


def _rcp(x):
    return pl.reciprocal(x, approx=True)


def _unpack(u):
    lo = pltpu.bitcast(u << 16, F32)
    hi = pltpu.bitcast(u & jnp.uint32(0xFFFF0000), F32)
    return lo, hi


def _ln(x):
    m = jnp.mean(x, axis=0, keepdims=True)
    c = x - m
    v = jnp.mean(c * c, axis=0, keepdims=True)
    return c * lax.rsqrt(v + 1e-5)


def _rhs7(b11, b12, b21, b22):
    return [v.astype(BF16) for v in (b11 + b22, b11, b12 - b22, b21 - b11, b22, b11 + b12, b21 + b22)]


def _lhs7(a11, a12, a21, a22):
    return [v.astype(BF16) for v in (a11 + a22, a21 + a22, a11, a22, a11 + a12, a21 - a11, a12 - a22)]


def _dual_softmax(p):
    ep = jnp.exp2(p - jnp.max(p, axis=0, keepdims=True))
    en = jnp.exp2(jnp.min(p, axis=0, keepdims=True) - p)
    ep = ep * _rcp(jnp.sum(ep, axis=0, keepdims=True))
    en = en * _rcp(jnp.sum(en, axis=0, keepdims=True))
    return jnp.concatenate([ep, en], axis=0).astype(BF16)


def _kernel(x_hbm, awqkv_hbm, awo_hbm, bwqkv_hbm, bwphi_ref, bwo_hbm, o_hbm,
            xio, stage, wos, tb, ws, xt, xs, k2, v2, os_, kvb, sems):
    def wcopy(src, col, slot, sem):
        return pltpu.make_async_copy(src.at[:, pl.ds(col * D, D)], stage.at[slot], sems.at[sem])

    cx = [pltpu.make_async_copy(x_hbm.at[:, pl.ds(c * 128, 128)], xio.at[c], sems.at[9 + c]) for c in range(8)]
    for c in cx:
        c.start()
    cps = [wcopy(awqkv_hbm, c, i, i + 1) for i, c in enumerate((1, 2, 0))]
    cwo = [pltpu.make_async_copy(awo_hbm.at[pl.ds(g * 256, 256), pl.ds(c * 128, 128)], wos.at[c * 4 + g], sems.at[4])
           for c in range(8) for g in range(4)]
    cps.append(None)
    srcs = [(bwqkv_hbm, 1), (bwqkv_hbm, 2), (bwqkv_hbm, 0), (bwo_hbm, 0)]
    cps += [wcopy(s, c, i + 3, i + 5) for i, (s, c) in enumerate(srcs)]
    for c in cps[:2]:
        c.start()

    xu = xio.bitcast(U32)

    def in_body(c, _):
        pltpu.make_async_copy(xio.at[0], xio.at[0], sems.at[9 + c]).wait()

        @pl.when(c == 5)
        def _():
            for cp in [cps[2]] + cwo:
                cp.start()
        rows = pl.ds(pl.multiple_of(c * 128, 128), 128)
        for m in range(8):
            lo, hi = _unpack(xu[c, pl.ds(m, 128, stride=8), :].T)
            xt[rows, m * 128:(m + 1) * 128] = lo
            xt[rows, (8 + m) * 128:(9 + m) * 128] = hi
    with jax.named_scope("loop_in"):
        lax.fori_loop(0, 8, in_body, None)
    for cp in cps[4:]:
        cp.start()

    def ln_tile(src, dst, x=None):
        y = _ln(xt[:, pl.ds(pl.multiple_of(src * NT, NT), NT)] if x is None else x)
        for i, v in enumerate(_rhs7(y[:512, :256], y[:512, 256:], y[512:, :256], y[512:, 256:])):
            xs[dst, i] = v
    with jax.named_scope("loop_ln"):
        lax.fori_loop(0, T, lambda t, c: ln_tile(t, t), None)

    def emit(mat, mc, r0, c0, *quads):
        for i, v in enumerate(_lhs7(*quads)):
            ws[mat * 2 + mc, i, r0:r0 + v.shape[0], c0:c0 + v.shape[1]] = v

    def prep_a(part, mc):
        tu = tb.bitcast(U32)
        for c in range(4):
            quads = []
            for j, (g, cc) in enumerate(((mc, c), (mc, c + 4), (mc + 2, c), (mc + 2, c + 4))):
                tb[j] = stage[part, cc * 128:(cc + 1) * 128, pl.ds(pl.multiple_of(g * 256, 256), 256)].T
                rows = []
                for e in range(16):
                    rows += list(_unpack(tu[j, pl.ds(e, 8, stride=16), :]))
                quads.append(jnp.concatenate(rows, 0))
            emit(part, mc, 0, c * 128, *quads)

    def prep_rest(mc):
        prep_a(2, mc)
        su = wos.bitcast(U32)
        for c in range(2):
            for gk in range(2):
                quads = []
                for cc, g in ((2 * mc + c, gk), (2 * mc + c, gk + 2), (2 * mc + c + 4, gk), (2 * mc + c + 4, gk + 2)):
                    rows = []
                    for e in range(16):
                        rows += list(_unpack(su[cc * 4 + g, pl.ds(e, 8, stride=16), :]))
                    quads.append(jnp.concatenate(rows, 0).T)
                emit(3, mc, c * 128, gk * 256, *quads)

    def prep_plain(slot, mat, mc):
        for c in range(4):
            quads = [stage[slot, cc * 128:(cc + 1) * 128, pl.ds(pl.multiple_of(g * 256, 256), 256)].T.astype(F32)
                     for g, cc in ((mc, c), (mc, c + 4), (mc + 2, c), (mc + 2, c + 4))]
            emit(mat, mc, 0, c * 128, *quads)

    def prep_fold(part, mc):
        zero = jnp.zeros((32, 32), F32)
        for gg in range(2):
            r = []
            for g in (mc, mc + 2):
                bd = jnp.concatenate(
                    [jnp.concatenate([bwphi_ref[8 * g + 4 * gg + i].astype(F32) if i == j else zero
                                      for j in range(4)], 1) for i in range(4)], 0).T.astype(BF16)
                wt = stage[3 + part, :, pl.ds(pl.multiple_of(g * 256 + gg * 128, 128), 128)].T
                r.append(_dot(bd, wt) * LOG2E)
            emit(4 + part, mc, gg * 128, 0, r[0][:, :512], r[0][:, 512:], r[1][:, :512], r[1][:, 512:])

    for part in range(2):
        cps[part].wait()
        with jax.named_scope("loop_pa"):
            lax.fori_loop(0, 2, lambda g, c: prep_a(part, g), None)
    for c in [cps[2]] + cwo:
        c.wait()
    with jax.named_scope("loop_pr"):
        lax.fori_loop(0, 2, lambda g, c: prep_rest(g), None)

    def sdot(mat, mc, rhs, k0=0, k1=512):
        p = [_dot(ws[mat * 2 + mc, i, :, k0:k1], rhs(i)[k0:k1, :]) for i in range(7)]
        return (jnp.concatenate([p[0] + p[3] - p[4] + p[6], p[2] + p[4]], 1),
                jnp.concatenate([p[1] + p[3], p[0] - p[1] + p[2] + p[5]], 1))

    def xdot(mat, mc, t):
        return sdot(mat, mc, lambda i: xs.at[t, i])

    def wo_part(mat, half):
        p = [sdot(mat, mc, lambda i: os_.at[i], *((0, 512) if mat == 7 else (half * 256, half * 256 + 256))) for mc in range(2)]
        return jnp.concatenate([p[0][0], p[1][0], p[0][1], p[1][1]], 0)

    def finish(mat, t, cols, part):
        x = part + wo_part(mat, 1)
        xt[:, cols] = x
        ln_tile(t, t, x)


    def emit_o(half, r0, c0, *quads):
        for i, v in enumerate(_rhs7(*quads)):
            os_[i, half * 256 + r0:half * 256 + r0 + v.shape[0], c0:c0 + v.shape[1]] = v

    def layer_a(it):
        def kv_body(t, _):
            cols = pl.ds(pl.multiple_of(jnp.int32(t) * NT, NT), NT)
            base = t * NB + 8 * (t * NB // 8)
            for part, dst in ((0, k2), (1, v2)):
                for mc in range(2):
                    for g, r in zip((mc, mc + 2), xdot(part, mc, t)):
                        for i in range(NB):
                            blk = r[:, i * 128:(i + 1) * 128]
                            dst[base + i + 8, g * 256:(g + 1) * 256] = blk
                            dst[base + i, g * 256:(g + 1) * 256] = pltpu.roll(blk, 1, 1)
            return 0
        with jax.named_scope("loop137"):
            kv_body(0, 0)

            @pl.when(it == 0)
            def _():
                for c in cps[4:]:
                    c.wait()
            for mc in range(2):
                prep_fold(0, mc)
                prep_fold(2, mc)
            kv_body(1, 0)

            def kv_prep(t, _):
                for mc in range(2):
                    prep_plain(2 * t, 2 * t + 1, mc)
                kv_body(t, 0)
            lax.fori_loop(2, T, kv_prep, None)

        def q_body(t, _):
            cols = pl.ds(pl.multiple_of(jnp.int32(t) * NT, NT), NT)
            base = t * NB + 8 * (t * NB // 8)
            m0 = t * NB % 8
            lane0 = lax.broadcasted_iota(jnp.int32, (8, 128), 1) == 0
            qs = [xdot(2, 0, t), xdot(2, 1, t)]
            for g in (0, 2, 1, 3):
                q = qs[g % 2][g // 2]
                if g == 1:
                    part = xt[:, cols] + wo_part(3, 0)
                if g < 2:
                    outs = []
                for i in range(NB):
                    lg = []
                    for w in range(W):
                        acc = None
                        for d in range(DH):
                            pr = (q[d * 8:(d + 1) * 8, i * 128:(i + 1) * 128]
                                  * k2[base + i + 8 - w, g * 256 + d * 8: g * 256 + (d + 1) * 8, :])
                            acc = pr if acc is None else acc + pr
                        acc = acc * (DH ** -0.5 * LOG2E)
                        if w > i:
                            acc = jnp.where(jnp.logical_and(lane0, m0 + i < w), -1e9 * LOG2E, acc)
                        lg.append(acc)
                    mx = lg[0]
                    for w in range(1, W):
                        mx = jnp.maximum(mx, lg[w])
                    es = [jnp.exp2(l - mx) for l in lg]
                    tot = es[0]
                    for w in range(1, W):
                        tot = tot + es[w]
                    inv = _rcp(tot)
                    ps = [e * inv for e in es]
                    rows = []
                    for d in range(DH):
                        acc = None
                        for w in range(W):
                            pr = ps[w] * v2[base + i + 8 - w, g * 256 + d * 8: g * 256 + (d + 1) * 8, :]
                            acc = pr if acc is None else acc + pr
                        rows.append(acc)
                    outs.append(jnp.concatenate(rows, 0))
                if g >= 2:
                    for i in range(2):
                        emit_o(g - 2, 0, i * 128, outs[i], outs[i + 2], outs[4 + i], outs[6 + i])
            finish(3, t, cols, part)
            return 0
        with jax.named_scope("loop178"):
            lax.fori_loop(0, T, q_body, 0)

    def layer_b():
        kvb[...] = jnp.zeros(kvb.shape, F32)

        def kv_body(t, _):
            cols = pl.ds(pl.multiple_of(jnp.int32(t) * NT, NT), NT)
            ones = jnp.ones((16, NT), BF16)
            ks = [xdot(4, mc, t) for mc in range(2)]
            vs = [xdot(5, mc, t) for mc in range(2)]
            for g in (0, 2, 1, 3):
                k = ks[g % 2][g // 2]
                v = vs[g % 2][g // 2].astype(BF16)
                for i in range(4):
                    phi = jnp.concatenate([_dual_softmax(k[i * 64:i * 64 + 32]),
                                           _dual_softmax(k[i * 64 + 32:i * 64 + 64])], 0)
                    lhs = jnp.concatenate([v[i * 64:(i + 1) * 64], ones], 0)
                    kvb[g * 4 + i] += _dot_nt(lhs, phi)
            return 0
        with jax.named_scope("loop195"):
            kv_body(0, 0)
            lax.fori_loop(1, T, kv_body, 0)
        r = lax.broadcasted_iota(jnp.int32, (80, 128), 0)
        c = lax.broadcasted_iota(jnp.int32, (80, 128), 1)
        keep = jnp.where(r < 64, r // 32, (r - 64) // 8) == c // 64
        for i in range(16):
            kvb[i] = jnp.where(keep, kvb[i], 0.0)

        def q_body(t, _):
            cols = pl.ds(pl.multiple_of(t * NT, NT), NT)
            qs = [xdot(6, 0, t), xdot(6, 1, t)]
            for g in (0, 2, 1, 3):
                q = qs[g % 2][g // 2]
                if g == 1:
                    part = xt[:, cols]
                if g < 2:
                    outs = []
                for i in range(4):
                    phi = jnp.concatenate([_dual_softmax(q[i * 64:i * 64 + 32]),
                                           _dual_softmax(q[i * 64 + 32:i * 64 + 64])], 0)
                    nd = _dot(kvb[g * 4 + i].astype(BF16), phi)
                    rows = []
                    for hh in range(2):
                        inv = _rcp(nd[64 + hh * 8:72 + hh * 8] + 1e-6)
                        rows += [nd[hh * 32 + j * 8: hh * 32 + (j + 1) * 8] * inv for j in range(4)]
                    outs.append(jnp.concatenate(rows, 0))
                    if g >= 2:
                        emit_o(g - 2, i * 64, 0, outs[i][:, :256], outs[i][:, 256:],
                               outs[4 + i][:, :256], outs[4 + i][:, 256:])
            finish(7, t, cols, part)
            return 0
        with jax.named_scope("loop217"):
            lax.fori_loop(0, T, q_body, 0)

    def pair(it, c):
        layer_a(it)
        layer_b()
        return c
    lax.fori_loop(0, 2, pair, 0)

    co = [pltpu.make_async_copy(xio.at[c], o_hbm.at[:, pl.ds(c * 128, 128)], sems.at[0]) for c in range(8)]

    def out_body(c, _):
        rows = pl.ds(pl.multiple_of(c * 128, 128), 128)
        for m in range(8):
            lo, hi = [pltpu.bitcast(xt[rows, b * 128:(b + 1) * 128].astype(BF16).astype(F32), U32)
                      for b in (m, 8 + m)]
            xu[c, pl.ds(m, 128, stride=8), :] = ((lo >> 16) | hi).T
        pltpu.make_async_copy(xio.at[c], o_hbm.at[:, pl.ds(pl.multiple_of(c * 128, 128), 128)], sems.at[0]).start()
    with jax.named_scope("loop_out"):
        lax.fori_loop(0, 8, out_body, None)
    for c in co:
        c.wait()


@jax.jit
def pallas_interleave_layers__sliding_local_dilated__linear_kernel_hedgehog__prompt_kernel(
    A_x, A_wqkv, A_wo, B_x, B_wqkv, B_w_phi, B_wo,
):
    hbm = pl.BlockSpec(memory_space=pl.ANY)
    out = pl.pallas_call(
        _kernel,
        out_shape=jax.ShapeDtypeStruct((S, D), BF16),
        in_specs=[hbm, hbm, hbm, hbm, pl.BlockSpec(memory_space=pltpu.VMEM), hbm],
        out_specs=hbm,
        scratch_shapes=[
            pltpu.VMEM((8, S, 128), BF16),
            pltpu.VMEM((7, D, D), BF16),
            pltpu.VMEM((32, 256, 128), BF16),
            pltpu.VMEM((4, 256, 128), BF16),
            pltpu.VMEM((16, 7, 256, 512), BF16),
            pltpu.VMEM((D, S), F32),
            pltpu.VMEM((T, 7, 512, 256), BF16),
            pltpu.VMEM((32, D, 128), F32),
            pltpu.VMEM((32, D, 128), F32),
            pltpu.VMEM((7, 512, 256), BF16),
            pltpu.VMEM((16, 80, 128), F32),
            pltpu.SemaphoreType.DMA((17,)),
        ],
        compiler_params=pltpu.CompilerParams(vmem_limit_bytes=126 * 1024 * 1024),
    )(A_x.reshape(S, D), A_wqkv, A_wo, B_wqkv, B_w_phi, B_wo)
    return out.reshape(1, S, D)
```

```python
import jax
import jax.numpy as jnp
from jax import lax
import jax.experimental.pallas as pl
import jax.experimental.pallas.tpu as pltpu

S, D, H, DH, W = 2048, 1024, 32, 32, 8
NT = 512
NB = NT // 128
T = S // NT
LOG2E = 1.4426950408889634
F32, BF16, U32 = jnp.float32, jnp.bfloat16, jnp.uint32


def _dot(a, b):
    return jnp.dot(a, b, preferred_element_type=F32)


def _dot_nt(a, b):
    return lax.dot_general(a, b, (((1,), (1,)), ((), ())), preferred_element_type=F32)


def _rcp(x):
    return pl.reciprocal(x, approx=True)


def _unpack(u):
    lo = pltpu.bitcast(u << 16, F32)
    hi = pltpu.bitcast(u & jnp.uint32(0xFFFF0000), F32)
    return lo, hi


def _ln(x):
    m = jnp.mean(x, axis=0, keepdims=True)
    c = x - m
    v = jnp.mean(c * c, axis=0, keepdims=True)
    return c * lax.rsqrt(v + 1e-5)


def _rhs7(b11, b12, b21, b22):
    return [v.astype(BF16) for v in (b11 + b22, b11, b12 - b22, b21 - b11, b22, b11 + b12, b21 + b22)]


def _lhs7(a11, a12, a21, a22):
    return [v.astype(BF16) for v in (a11 + a22, a21 + a22, a11, a22, a11 + a12, a21 - a11, a12 - a22)]


def _dual_softmax(p):
    ep = jnp.exp2(p - jnp.max(p, axis=0, keepdims=True))
    en = jnp.exp2(jnp.min(p, axis=0, keepdims=True) - p)
    ep = ep * _rcp(jnp.sum(ep, axis=0, keepdims=True))
    en = en * _rcp(jnp.sum(en, axis=0, keepdims=True))
    return jnp.concatenate([ep, en], axis=0).astype(BF16)


def _kernel(x_hbm, awqkv_hbm, awo_hbm, bwqkv_hbm, bwphi_ref, bwo_hbm, o_hbm,
            xio, stage, wos, tb, ws, xt, xs, k2, v2, os_, os2, kvb, sems):
    def wcopy(src, col, slot, sem):
        return pltpu.make_async_copy(src.at[:, pl.ds(col * D, D)], stage.at[slot], sems.at[sem])

    cx = [pltpu.make_async_copy(x_hbm.at[:, pl.ds(c * 128, 128)], xio.at[c], sems.at[9 + c]) for c in range(8)]
    for c in cx:
        c.start()
    cps = [wcopy(awqkv_hbm, c, i, i + 1) for i, c in enumerate((1, 2, 0))]
    cwo = [pltpu.make_async_copy(awo_hbm.at[pl.ds(g * 256, 256), pl.ds(c * 128, 128)], wos.at[c * 4 + g], sems.at[4])
           for c in range(8) for g in range(4)]
    cps.append(None)
    srcs = [(bwqkv_hbm, 1), (bwqkv_hbm, 2), (bwqkv_hbm, 0), (bwo_hbm, 0)]
    cps += [wcopy(s, c, i + 3, i + 5) for i, (s, c) in enumerate(srcs)]
    for c in cps[:2]:
        c.start()

    xu = xio.bitcast(U32)

    def in_body(c, _):
        pltpu.make_async_copy(xio.at[0], xio.at[0], sems.at[9 + c]).wait()

        @pl.when(c == 5)
        def _():
            for cp in [cps[2]] + cwo:
                cp.start()
        rows = pl.ds(pl.multiple_of(c * 128, 128), 128)
        for m in range(8):
            lo, hi = _unpack(xu[c, pl.ds(m, 128, stride=8), :].T)
            xt[rows, m * 128:(m + 1) * 128] = lo
            xt[rows, (8 + m) * 128:(9 + m) * 128] = hi
    with jax.named_scope("loop_in"):
        lax.fori_loop(0, 8, in_body, None)
    for cp in cps[4:]:
        cp.start()

    def ln_tile(src, dst, x=None):
        y = _ln(xt[:, pl.ds(pl.multiple_of(src * NT, NT), NT)] if x is None else x)
        for i, v in enumerate(_rhs7(y[:512, :256], y[:512, 256:], y[512:, :256], y[512:, 256:])):
            xs[dst, i] = v
    with jax.named_scope("loop_ln"):
        lax.fori_loop(0, T, lambda t, c: ln_tile(t, t), None)

    def emit(mat, mc, r0, c0, *quads):
        for i, v in enumerate(_lhs7(*quads)):
            ws[mat * 2 + mc, i, r0:r0 + v.shape[0], c0:c0 + v.shape[1]] = v

    def prep_a(part, mc):
        tu = tb.bitcast(U32)
        for c in range(4):
            quads = []
            for j, (g, cc) in enumerate(((mc, c), (mc, c + 4), (mc + 2, c), (mc + 2, c + 4))):
                tb[j] = stage[part, cc * 128:(cc + 1) * 128, pl.ds(pl.multiple_of(g * 256, 256), 256)].T
                rows = []
                for e in range(16):
                    rows += list(_unpack(tu[j, pl.ds(e, 8, stride=16), :]))
                quads.append(jnp.concatenate(rows, 0))
            emit(part, mc, 0, c * 128, *quads)

    def prep_rest(mc):
        prep_a(2, mc)
        su = wos.bitcast(U32)
        for c in range(2):
            for gk in range(2):
                quads = []
                for cc, g in ((2 * mc + c, gk), (2 * mc + c, gk + 2), (2 * mc + c + 4, gk), (2 * mc + c + 4, gk + 2)):
                    rows = []
                    for e in range(16):
                        rows += list(_unpack(su[cc * 4 + g, pl.ds(e, 8, stride=16), :]))
                    quads.append(jnp.concatenate(rows, 0).T)
                emit(3, mc, c * 128, gk * 256, *quads)

    def prep_plain(slot, mat, mc):
        for c in range(4):
            quads = [stage[slot, cc * 128:(cc + 1) * 128, pl.ds(pl.multiple_of(g * 256, 256), 256)].T.astype(F32)
                     for g, cc in ((mc, c), (mc, c + 4), (mc + 2, c), (mc + 2, c + 4))]
            emit(mat, mc, 0, c * 128, *quads)

    def prep_fold(part, mc):
        zero = jnp.zeros((32, 32), F32)
        for gg in range(2):
            r = []
            for g in (mc, mc + 2):
                bd = jnp.concatenate(
                    [jnp.concatenate([bwphi_ref[8 * g + 4 * gg + i].astype(F32) if i == j else zero
                                      for j in range(4)], 1) for i in range(4)], 0).T.astype(BF16)
                wt = stage[3 + part, :, pl.ds(pl.multiple_of(g * 256 + gg * 128, 128), 128)].T
                r.append(_dot(bd, wt) * LOG2E)
            emit(4 + part, mc, gg * 128, 0, r[0][:, :512], r[0][:, 512:], r[1][:, :512], r[1][:, 512:])

    for part in range(2):
        cps[part].wait()
        with jax.named_scope("loop_pa"):
            lax.fori_loop(0, 2, lambda g, c: prep_a(part, g), None)
    for c in [cps[2]] + cwo:
        c.wait()
    with jax.named_scope("loop_pr"):
        lax.fori_loop(0, 2, lambda g, c: prep_rest(g), None)

    def sdot(mat, mc, rhs, k0=0, k1=512):
        p = [_dot(ws[mat * 2 + mc, i, :, k0:k1], rhs(i)[k0:k1, :]) for i in range(7)]
        return (jnp.concatenate([p[0] + p[3] - p[4] + p[6], p[2] + p[4]], 1),
                jnp.concatenate([p[1] + p[3], p[0] - p[1] + p[2] + p[5]], 1))

    def xdot(mat, mc, t):
        return sdot(mat, mc, lambda i: xs.at[t, i])

    def wo_part(mat, half):
        p = [sdot(mat, mc, lambda i: os_.at[i], *((0, 512) if mat == 7 else (half * 256, half * 256 + 256))) for mc in range(2)]
        return jnp.concatenate([p[0][0], p[1][0], p[0][1], p[1][1]], 0)

    def finish(mat, t, cols, part):
        x = part + wo_part(mat, 1)
        xt[:, cols] = x
        ln_tile(t, t, x)


    def emit_o(half, r0, c0, *quads, dst=os_):
        for i, v in enumerate(_rhs7(*quads)):
            dst[i, half * 256 + r0:half * 256 + r0 + v.shape[0], c0:c0 + v.shape[1]] = v

    def layer_a(it):
        def kv_body(t, _):
            cols = pl.ds(pl.multiple_of(jnp.int32(t) * NT, NT), NT)
            base = t * NB + 8 * (t * NB // 8)
            for part, dst in ((0, k2), (1, v2)):
                for mc in range(2):
                    for g, r in zip((mc, mc + 2), xdot(part, mc, t)):
                        for i in range(NB):
                            blk = r[:, i * 128:(i + 1) * 128]
                            dst[base + i + 8, g * 256:(g + 1) * 256] = blk
                            dst[base + i, g * 256:(g + 1) * 256] = pltpu.roll(blk, 1, 1)
            return 0
        with jax.named_scope("loop137"):
            kv_body(0, 0)

            @pl.when(it == 0)
            def _():
                for c in cps[4:]:
                    c.wait()
            for mc in range(2):
                prep_fold(0, mc)
                prep_fold(2, mc)
            kv_body(1, 0)

            def kv_prep(t, _):
                for mc in range(2):
                    prep_plain(2 * t, 2 * t + 1, mc)
                kv_body(t, 0)
            lax.fori_loop(2, T, kv_prep, None)

        def q_body(t, _):
            cols = pl.ds(pl.multiple_of(jnp.int32(t) * NT, NT), NT)
            base = t * NB + 8 * (t * NB // 8)
            m0 = t * NB % 8
            lane0 = lax.broadcasted_iota(jnp.int32, (8, 128), 1) == 0
            qs = [xdot(2, 0, t), xdot(2, 1, t)]
            for g in (0, 2, 1, 3):
                q = qs[g % 2][g // 2]
                if g == 1:
                    part = xt[:, cols] + wo_part(3, 0)
                if g < 2:
                    outs = []
                for i in range(NB):
                    lg = []
                    for w in range(W):
                        acc = None
                        for d in range(DH):
                            pr = (q[d * 8:(d + 1) * 8, i * 128:(i + 1) * 128]
                                  * k2[base + i + 8 - w, g * 256 + d * 8: g * 256 + (d + 1) * 8, :])
                            acc = pr if acc is None else acc + pr
                        acc = acc * (DH ** -0.5 * LOG2E)
                        if w > i:
                            acc = jnp.where(jnp.logical_and(lane0, m0 + i < w), -1e9 * LOG2E, acc)
                        lg.append(acc)
                    mx = lg[0]
                    for w in range(1, W):
                        mx = jnp.maximum(mx, lg[w])
                    es = [jnp.exp2(l - mx) for l in lg]
                    tot = es[0]
                    for w in range(1, W):
                        tot = tot + es[w]
                    inv = _rcp(tot)
                    ps = [e * inv for e in es]
                    rows = []
                    for d in range(DH):
                        acc = None
                        for w in range(W):
                            pr = ps[w] * v2[base + i + 8 - w, g * 256 + d * 8: g * 256 + (d + 1) * 8, :]
                            acc = pr if acc is None else acc + pr
                        rows.append(acc)
                    outs.append(jnp.concatenate(rows, 0))
                if g >= 2:
                    for i in range(2):
                        emit_o(g - 2, 0, i * 128, outs[i], outs[i + 2], outs[4 + i], outs[6 + i])
            finish(3, t, cols, part)
            return 0
        with jax.named_scope("loop178"):
            lax.fori_loop(0, T, q_body, 0)

    def layer_b():
        kvb[...] = jnp.zeros(kvb.shape, F32)

        def kv_body(t, _):
            cols = pl.ds(pl.multiple_of(jnp.int32(t) * NT, NT), NT)
            ones = jnp.ones((16, NT), BF16)
            ks = [xdot(4, mc, t) for mc in range(2)]
            vs = [xdot(5, mc, t) for mc in range(2)]
            for g in (0, 2, 1, 3):
                k = ks[g % 2][g // 2]
                v = vs[g % 2][g // 2].astype(BF16)
                for i in range(4):
                    phi = jnp.concatenate([_dual_softmax(k[i * 64:i * 64 + 32]),
                                           _dual_softmax(k[i * 64 + 32:i * 64 + 64])], 0)
                    lhs = jnp.concatenate([v[i * 64:(i + 1) * 64], ones], 0)
                    kvb[g * 4 + i] += _dot_nt(lhs, phi)
            return 0
        with jax.named_scope("loop195"):
            kv_body(0, 0)
            lax.fori_loop(1, T, kv_body, 0)
        r = lax.broadcasted_iota(jnp.int32, (80, 128), 0)
        c = lax.broadcasted_iota(jnp.int32, (80, 128), 1)
        keep = jnp.where(r < 64, r // 32, (r - 64) // 8) == c // 64
        for i in range(16):
            kvb[i] = jnp.where(keep, kvb[i], 0.0)

        def chunk(t, mc, qq):
            for i in range(4):
                outs = []
                for j in range(2):
                    q = qq[j]
                    phi = jnp.concatenate([_dual_softmax(q[i * 64:i * 64 + 32]),
                                           _dual_softmax(q[i * 64 + 32:i * 64 + 64])], 0)
                    nd = _dot(kvb[(mc + 2 * j) * 4 + i].astype(BF16), phi)
                    rows = []
                    for hh in range(2):
                        inv = _rcp(nd[64 + hh * 8:72 + hh * 8] + 1e-6)
                        rows += [nd[hh * 32 + r * 8: hh * 32 + (r + 1) * 8] * inv for r in range(4)]
                    outs.append(jnp.concatenate(rows, 0))
                emit_o(mc, i * 64, 0, outs[0][:, :256], outs[0][:, 256:], outs[1][:, :256], outs[1][:, 256:],
                       dst=(os_, os2)[t % 2])

        with jax.named_scope("loop217"):
            q0 = xdot(6, 0, 0)
            q1 = xdot(6, 1, 0)
            chunk(0, 0, q0)
            for t in range(T):
                if t + 1 < T:
                    q0 = xdot(6, 0, t + 1)
                chunk(t, 1, q1)
                if t + 1 < T:
                    q1 = xdot(6, 1, t + 1)
                src = (os_, os2)[t % 2]
                p = [sdot(7, mc, lambda i: src.at[i]) for mc in range(2)]
                cols = slice(t * NT, (t + 1) * NT)
                x = xt[:, cols] + jnp.concatenate([p[0][0], p[1][0], p[0][1], p[1][1]], 0)
                xt[:, cols] = x
                ln_tile(t, t, x)
                if t + 1 < T:
                    chunk(t + 1, 0, q0)

    def pair(it, c):
        layer_a(it)
        layer_b()
        return c
    lax.fori_loop(0, 2, pair, 0)

    co = [pltpu.make_async_copy(xio.at[c], o_hbm.at[:, pl.ds(c * 128, 128)], sems.at[0]) for c in range(8)]

    def out_body(c, _):
        rows = pl.ds(pl.multiple_of(c * 128, 128), 128)
        for m in range(8):
            lo, hi = [pltpu.bitcast(xt[rows, b * 128:(b + 1) * 128].astype(BF16).astype(F32), U32)
                      for b in (m, 8 + m)]
            xu[c, pl.ds(m, 128, stride=8), :] = ((lo >> 16) | hi).T
        pltpu.make_async_copy(xio.at[c], o_hbm.at[:, pl.ds(pl.multiple_of(c * 128, 128), 128)], sems.at[0]).start()
    with jax.named_scope("loop_out"):
        lax.fori_loop(0, 8, out_body, None)
    for c in co:
        c.wait()


@jax.jit
def pallas_interleave_layers__sliding_local_dilated__linear_kernel_hedgehog__prompt_kernel(
    A_x, A_wqkv, A_wo, B_x, B_wqkv, B_w_phi, B_wo,
):
    hbm = pl.BlockSpec(memory_space=pl.ANY)
    out = pl.pallas_call(
        _kernel,
        out_shape=jax.ShapeDtypeStruct((S, D), BF16),
        in_specs=[hbm, hbm, hbm, hbm, pl.BlockSpec(memory_space=pltpu.VMEM), hbm],
        out_specs=hbm,
        scratch_shapes=[
            pltpu.VMEM((8, S, 128), BF16),
            pltpu.VMEM((7, D, D), BF16),
            pltpu.VMEM((32, 256, 128), BF16),
            pltpu.VMEM((4, 256, 128), BF16),
            pltpu.VMEM((16, 7, 256, 512), BF16),
            pltpu.VMEM((D, S), F32),
            pltpu.VMEM((T, 7, 512, 256), BF16),
            pltpu.VMEM((32, D, 128), F32),
            pltpu.VMEM((32, D, 128), F32),
            pltpu.VMEM((7, 512, 256), BF16),
            pltpu.VMEM((7, 512, 256), BF16),
            pltpu.VMEM((16, 80, 128), F32),
            pltpu.SemaphoreType.DMA((17,)),
        ],
        compiler_params=pltpu.CompilerParams(vmem_limit_bytes=126 * 1024 * 1024),
    )(A_x.reshape(S, D), A_wqkv, A_wo, B_wqkv, B_w_phi, B_wo)
    return out.reshape(1, S, D)
```

```python
import jax
import jax.numpy as jnp
from jax import lax
import jax.experimental.pallas as pl
import jax.experimental.pallas.tpu as pltpu

S, D, H, DH, W = 2048, 1024, 32, 32, 8
NT = 512
NB = NT // 128
T = S // NT
LOG2E = 1.4426950408889634
F32, BF16, U32 = jnp.float32, jnp.bfloat16, jnp.uint32


def _dot(a, b):
    return jnp.dot(a, b, preferred_element_type=F32)


def _dot_nt(a, b):
    return lax.dot_general(a, b, (((1,), (1,)), ((), ())), preferred_element_type=F32)


def _rcp(x):
    return pl.reciprocal(x, approx=True)


def _unpack(u):
    lo = pltpu.bitcast(u << 16, F32)
    hi = pltpu.bitcast(u & jnp.uint32(0xFFFF0000), F32)
    return lo, hi


def _ln(x):
    m = jnp.mean(x, axis=0, keepdims=True)
    c = x - m
    v = jnp.mean(c * c, axis=0, keepdims=True)
    return c * lax.rsqrt(v + 1e-5)


def _rhs7(b11, b12, b21, b22):
    return [v.astype(BF16) for v in (b11 + b22, b11, b12 - b22, b21 - b11, b22, b11 + b12, b21 + b22)]


def _lhs7(a11, a12, a21, a22):
    return [v.astype(BF16) for v in (a11 + a22, a21 + a22, a11, a22, a11 + a12, a21 - a11, a12 - a22)]


def _dual_softmax(p):
    ep = jnp.exp2(p - jnp.max(p, axis=0, keepdims=True))
    en = jnp.exp2(jnp.min(p, axis=0, keepdims=True) - p)
    ep = ep * _rcp(jnp.sum(ep, axis=0, keepdims=True))
    en = en * _rcp(jnp.sum(en, axis=0, keepdims=True))
    return jnp.concatenate([ep, en], axis=0).astype(BF16)


def _kernel(x_hbm, awqkv_hbm, awo_hbm, bwqkv_hbm, bwphi_ref, bwo_hbm, o_hbm,
            xio, stage, wos, tb, ws, xt, xs, k2, v2, os_, os2, kvb, sems):
    def wcopy(src, col, slot, sem):
        return pltpu.make_async_copy(src.at[:, pl.ds(col * D, D)], stage.at[slot], sems.at[sem])

    cx = [pltpu.make_async_copy(x_hbm.at[:, pl.ds(c * 128, 128)], xio.at[c], sems.at[9 + c]) for c in range(8)]
    cps = [wcopy(awqkv_hbm, c, i, i + 1) for i, c in enumerate((1, 2, 0))]
    cwo = [pltpu.make_async_copy(awo_hbm.at[pl.ds(g * 256, 256), pl.ds(c * 128, 128)], wos.at[c * 4 + g], sems.at[4])
           for c in range(8) for g in range(4)]
    cps.append(None)
    srcs = [(bwqkv_hbm, 1), (bwqkv_hbm, 2), (bwqkv_hbm, 0), (bwo_hbm, 0)]
    cps += [wcopy(s, c, i + 3, i + 5) for i, (s, c) in enumerate(srcs)]
    for c in cps[:1] + cx + cps[1:2]:
        c.start()

    xu = xio.bitcast(U32)

    def in_body(c, _):
        pltpu.make_async_copy(xio.at[0], xio.at[0], sems.at[9 + c]).wait()

        @pl.when(c == 3)
        def _():
            for cp in [cps[2]] + cwo:
                cp.start()
        rows = pl.ds(pl.multiple_of(c * 128, 128), 128)
        for m in range(8):
            lo, hi = _unpack(xu[c, pl.ds(m, 128, stride=8), :].T)
            xt[rows, m * 128:(m + 1) * 128] = lo
            xt[rows, (8 + m) * 128:(9 + m) * 128] = hi
    def ln_tile(src, dst, x=None):
        y = _ln(xt[:, pl.ds(pl.multiple_of(src * NT, NT), NT)] if x is None else x)
        for i, v in enumerate(_rhs7(y[:512, :256], y[:512, 256:], y[512:, :256], y[512:, 256:])):
            xs[dst, i] = v

    def load_x():
        with jax.named_scope("loop_in"):
            lax.fori_loop(0, 8, in_body, None)
        for cp in cps[4:]:
            cp.start()
        with jax.named_scope("loop_ln"):
            lax.fori_loop(0, T, lambda t, c: ln_tile(t, t), None)

    def emit(mat, mc, r0, c0, *quads):
        for i, v in enumerate(_lhs7(*quads)):
            ws[mat * 2 + mc, i, r0:r0 + v.shape[0], c0:c0 + v.shape[1]] = v

    def prep_a(part, mc):
        tu = tb.bitcast(U32)
        for c in range(4):
            quads = []
            for j, (g, cc) in enumerate(((mc, c), (mc, c + 4), (mc + 2, c), (mc + 2, c + 4))):
                tb[j] = stage[part, cc * 128:(cc + 1) * 128, pl.ds(pl.multiple_of(g * 256, 256), 256)].T
                rows = []
                for e in range(16):
                    rows += list(_unpack(tu[j, pl.ds(e, 8, stride=16), :]))
                quads.append(jnp.concatenate(rows, 0))
            emit(part, mc, 0, c * 128, *quads)

    def prep_rest(mc):
        prep_a(2, mc)
        su = wos.bitcast(U32)
        for c in range(2):
            for gk in range(2):
                quads = []
                for cc, g in ((2 * mc + c, gk), (2 * mc + c, gk + 2), (2 * mc + c + 4, gk), (2 * mc + c + 4, gk + 2)):
                    rows = []
                    for e in range(16):
                        rows += list(_unpack(su[cc * 4 + g, pl.ds(e, 8, stride=16), :]))
                    quads.append(jnp.concatenate(rows, 0).T)
                emit(3, mc, c * 128, gk * 256, *quads)

    def prep_plain(slot, mat, mc):
        for c in range(4):
            quads = [stage[slot, cc * 128:(cc + 1) * 128, pl.ds(pl.multiple_of(g * 256, 256), 256)].T.astype(F32)
                     for g, cc in ((mc, c), (mc, c + 4), (mc + 2, c), (mc + 2, c + 4))]
            emit(mat, mc, 0, c * 128, *quads)

    def prep_fold(part, mc):
        zero = jnp.zeros((32, 32), F32)
        for gg in range(2):
            r = []
            for g in (mc, mc + 2):
                bd = jnp.concatenate(
                    [jnp.concatenate([bwphi_ref[8 * g + 4 * gg + i].astype(F32) if i == j else zero
                                      for j in range(4)], 1) for i in range(4)], 0).T.astype(BF16)
                wt = stage[3 + part, :, pl.ds(pl.multiple_of(g * 256 + gg * 128, 128), 128)].T
                r.append(_dot(bd, wt) * LOG2E)
            emit(4 + part, mc, gg * 128, 0, r[0][:, :512], r[0][:, 512:], r[1][:, :512], r[1][:, 512:])

    def first(part):
        cps[part].wait()
        with jax.named_scope("loop_pa"):
            lax.fori_loop(0, 2, lambda g, c: prep_a(part, g), None)
    first(0)
    load_x()
    first(1)
    for c in [cps[2]] + cwo:
        c.wait()
    with jax.named_scope("loop_pr"):
        lax.fori_loop(0, 2, lambda g, c: prep_rest(g), None)

    def sdot(mat, mc, rhs, k0=0, k1=512):
        p = [_dot(ws[mat * 2 + mc, i, :, k0:k1], rhs(i)[k0:k1, :]) for i in range(7)]
        return (jnp.concatenate([p[0] + p[3] - p[4] + p[6], p[2] + p[4]], 1),
                jnp.concatenate([p[1] + p[3], p[0] - p[1] + p[2] + p[5]], 1))

    def xdot(mat, mc, t):
        return sdot(mat, mc, lambda i: xs.at[t, i])

    def wo_part(mat, half):
        p = [sdot(mat, mc, lambda i: os_.at[i], *((0, 512) if mat == 7 else (half * 256, half * 256 + 256))) for mc in range(2)]
        return jnp.concatenate([p[0][0], p[1][0], p[0][1], p[1][1]], 0)

    def finish(mat, t, cols, part):
        x = part + wo_part(mat, 1)
        xt[:, cols] = x
        ln_tile(t, t, x)


    def emit_o(half, r0, c0, *quads, dst=os_):
        for i, v in enumerate(_rhs7(*quads)):
            dst[i, half * 256 + r0:half * 256 + r0 + v.shape[0], c0:c0 + v.shape[1]] = v

    def layer_a(it):
        def kv_body(t, _):
            cols = pl.ds(pl.multiple_of(jnp.int32(t) * NT, NT), NT)
            base = t * NB + 8 * (t * NB // 8)
            for part, dst in ((0, k2), (1, v2)):
                for mc in range(2):
                    for g, r in zip((mc, mc + 2), xdot(part, mc, t)):
                        for i in range(NB):
                            blk = r[:, i * 128:(i + 1) * 128]
                            dst[base + i + 8, g * 256:(g + 1) * 256] = blk
                            dst[base + i, g * 256:(g + 1) * 256] = pltpu.roll(blk, 1, 1)
            return 0
        with jax.named_scope("loop137"):
            lax.fori_loop(0, T, kv_body, 0)

        @pl.when(it == 0)
        def _():
            for c in cps[4:]:
                c.wait()

            def prep_b(mc, _):
                prep_fold(0, mc)
                prep_fold(2, mc)
                prep_plain(4, 5, mc)
                prep_plain(6, 7, mc)
            lax.fori_loop(0, 2, prep_b, None)

        def q_body(t, _):
            cols = pl.ds(pl.multiple_of(jnp.int32(t) * NT, NT), NT)
            base = t * NB + 8 * (t * NB // 8)
            m0 = t * NB % 8
            lane0 = lax.broadcasted_iota(jnp.int32, (8, 128), 1) == 0
            qs = [xdot(2, 0, t), xdot(2, 1, t)]
            for g in (0, 2, 1, 3):
                q = qs[g % 2][g // 2]
                if g == 1:
                    part = xt[:, cols] + wo_part(3, 0)
                if g < 2:
                    outs = []
                for i in range(NB):
                    lg = []
                    for w in range(W):
                        acc = None
                        for d in range(DH):
                            pr = (q[d * 8:(d + 1) * 8, i * 128:(i + 1) * 128]
                                  * k2[base + i + 8 - w, g * 256 + d * 8: g * 256 + (d + 1) * 8, :])
                            acc = pr if acc is None else acc + pr
                        acc = acc * (DH ** -0.5 * LOG2E)
                        if w > i:
                            acc = jnp.where(jnp.logical_and(lane0, m0 + i < w), -1e9 * LOG2E, acc)
                        lg.append(acc)
                    mx = lg[0]
                    for w in range(1, W):
                        mx = jnp.maximum(mx, lg[w])
                    es = [jnp.exp2(l - mx) for l in lg]
                    tot = es[0]
                    for w in range(1, W):
                        tot = tot + es[w]
                    inv = _rcp(tot)
                    ps = [e * inv for e in es]
                    rows = []
                    for d in range(DH):
                        acc = None
                        for w in range(W):
                            pr = ps[w] * v2[base + i + 8 - w, g * 256 + d * 8: g * 256 + (d + 1) * 8, :]
                            acc = pr if acc is None else acc + pr
                        rows.append(acc)
                    outs.append(jnp.concatenate(rows, 0))
                if g >= 2:
                    for i in range(2):
                        emit_o(g - 2, 0, i * 128, outs[i], outs[i + 2], outs[4 + i], outs[6 + i])
            finish(3, t, cols, part)
            return 0
        with jax.named_scope("loop178"):
            lax.fori_loop(0, T, q_body, 0)

    def layer_b():
        kvb[...] = jnp.zeros(kvb.shape, F32)

        def kv_body(t, _):
            cols = pl.ds(pl.multiple_of(jnp.int32(t) * NT, NT), NT)
            ones = jnp.ones((16, NT), BF16)
            ks = [xdot(4, mc, t) for mc in range(2)]
            vs = [xdot(5, mc, t) for mc in range(2)]
            for g in (0, 2, 1, 3):
                k = ks[g % 2][g // 2]
                v = vs[g % 2][g // 2].astype(BF16)
                for i in range(4):
                    phi = jnp.concatenate([_dual_softmax(k[i * 64:i * 64 + 32]),
                                           _dual_softmax(k[i * 64 + 32:i * 64 + 64])], 0)
                    lhs = jnp.concatenate([v[i * 64:(i + 1) * 64], ones], 0)
                    kvb[g * 4 + i] += _dot_nt(lhs, phi)
            return 0
        with jax.named_scope("loop195"):
            kv_body(0, 0)
            lax.fori_loop(1, T, kv_body, 0)
        r = lax.broadcasted_iota(jnp.int32, (80, 128), 0)
        c = lax.broadcasted_iota(jnp.int32, (80, 128), 1)
        keep = jnp.where(r < 64, r // 32, (r - 64) // 8) == c // 64
        for i in range(16):
            kvb[i] = jnp.where(keep, kvb[i], 0.0)

        def chunk(t, mc, qq):
            for i in range(4):
                outs = []
                for j in range(2):
                    q = qq[j]
                    phi = jnp.concatenate([_dual_softmax(q[i * 64:i * 64 + 32]),
                                           _dual_softmax(q[i * 64 + 32:i * 64 + 64])], 0)
                    nd = _dot(kvb[(mc + 2 * j) * 4 + i].astype(BF16), phi)
                    rows = []
                    for hh in range(2):
                        inv = _rcp(nd[64 + hh * 8:72 + hh * 8] + 1e-6)
                        rows += [nd[hh * 32 + r * 8: hh * 32 + (r + 1) * 8] * inv for r in range(4)]
                    outs.append(jnp.concatenate(rows, 0))
                emit_o(mc, i * 64, 0, outs[0][:, :256], outs[0][:, 256:], outs[1][:, :256], outs[1][:, 256:],
                       dst=(os_, os2)[t % 2])

        with jax.named_scope("loop217"):
            q0 = xdot(6, 0, 0)
            q1 = xdot(6, 1, 0)
            chunk(0, 0, q0)
            for t in range(T):
                if t + 1 < T:
                    q0 = xdot(6, 0, t + 1)
                chunk(t, 1, q1)
                if t + 1 < T:
                    q1 = xdot(6, 1, t + 1)
                src = (os_, os2)[t % 2]
                p = [sdot(7, mc, lambda i: src.at[i]) for mc in range(2)]
                cols = slice(t * NT, (t + 1) * NT)
                x = xt[:, cols] + jnp.concatenate([p[0][0], p[1][0], p[0][1], p[1][1]], 0)
                xt[:, cols] = x
                ln_tile(t, t, x)
                if t + 1 < T:
                    chunk(t + 1, 0, q0)

    def pair(it, c):
        layer_a(it)
        layer_b()
        return c
    lax.fori_loop(0, 2, pair, 0)

    co = [pltpu.make_async_copy(xio.at[c], o_hbm.at[:, pl.ds(c * 128, 128)], sems.at[0]) for c in range(8)]

    def out_body(c, _):
        rows = pl.ds(pl.multiple_of(c * 128, 128), 128)
        for m in range(8):
            lo, hi = [pltpu.bitcast(xt[rows, b * 128:(b + 1) * 128].astype(BF16).astype(F32), U32)
                      for b in (m, 8 + m)]
            xu[c, pl.ds(m, 128, stride=8), :] = ((lo >> 16) | hi).T
        pltpu.make_async_copy(xio.at[c], o_hbm.at[:, pl.ds(pl.multiple_of(c * 128, 128), 128)], sems.at[0]).start()
    with jax.named_scope("loop_out"):
        lax.fori_loop(0, 8, out_body, None)
    for c in co:
        c.wait()


@jax.jit
def pallas_interleave_layers__sliding_local_dilated__linear_kernel_hedgehog__prompt_kernel(
    A_x, A_wqkv, A_wo, B_x, B_wqkv, B_w_phi, B_wo,
):
    hbm = pl.BlockSpec(memory_space=pl.ANY)
    out = pl.pallas_call(
        _kernel,
        out_shape=jax.ShapeDtypeStruct((S, D), BF16),
        in_specs=[hbm, hbm, hbm, hbm, pl.BlockSpec(memory_space=pltpu.VMEM), hbm],
        out_specs=hbm,
        scratch_shapes=[
            pltpu.VMEM((8, S, 128), BF16),
            pltpu.VMEM((7, D, D), BF16),
            pltpu.VMEM((32, 256, 128), BF16),
            pltpu.VMEM((4, 256, 128), BF16),
            pltpu.VMEM((16, 7, 256, 512), BF16),
            pltpu.VMEM((D, S), F32),
            pltpu.VMEM((T, 7, 512, 256), BF16),
            pltpu.VMEM((32, D, 128), F32),
            pltpu.VMEM((32, D, 128), F32),
            pltpu.VMEM((7, 512, 256), BF16),
            pltpu.VMEM((7, 512, 256), BF16),
            pltpu.VMEM((16, 80, 128), F32),
            pltpu.SemaphoreType.DMA((17,)),
        ],
        compiler_params=pltpu.CompilerParams(vmem_limit_bytes=126 * 1024 * 1024),
    )(A_x.reshape(S, D), A_wqkv, A_wo, B_wqkv, B_w_phi, B_wo)
    return out.reshape(1, S, D)
```

```python
import jax
import jax.numpy as jnp
from jax import lax
import jax.experimental.pallas as pl
import jax.experimental.pallas.tpu as pltpu

S, D, H, DH, W = 2048, 1024, 32, 32, 8
NT = 512
NB = NT // 128
T = S // NT
LOG2E = 1.4426950408889634
F32, BF16, U32 = jnp.float32, jnp.bfloat16, jnp.uint32


def _dot(a, b):
    return jnp.dot(a, b, preferred_element_type=F32)


def _dot_nt(a, b):
    return lax.dot_general(a, b, (((1,), (1,)), ((), ())), preferred_element_type=F32)


def _rcp(x):
    return pl.reciprocal(x, approx=True)


def _unpack(u):
    lo = pltpu.bitcast(u << 16, F32)
    hi = pltpu.bitcast(u & jnp.uint32(0xFFFF0000), F32)
    return lo, hi


def _rhs7(b11, b12, b21, b22):
    return [v.astype(BF16) for v in (b11 + b22, b11, b12 - b22, b21 - b11, b22, b11 + b12, b21 + b22)]


def _lhs7(a11, a12, a21, a22):
    return [v.astype(BF16) for v in (a11 + a22, a21 + a22, a11, a22, a11 + a12, a21 - a11, a12 - a22)]


def _dual_softmax(p):
    ep = jnp.exp2(p - jnp.max(p, axis=0, keepdims=True))
    en = jnp.exp2(jnp.min(p, axis=0, keepdims=True) - p)
    ep = ep * _rcp(jnp.sum(ep, axis=0, keepdims=True))
    en = en * _rcp(jnp.sum(en, axis=0, keepdims=True))
    return jnp.concatenate([ep, en], axis=0).astype(BF16)


def _kernel(x_hbm, awqkv_hbm, awo_hbm, bwqkv_hbm, bwphi_ref, bwo_hbm, o_hbm,
            xio, stage, wos, tb, ws, xt, xs, k2, v2, os_, os2, kvb, sems):
    def wcopy(src, col, slot, sem):
        return pltpu.make_async_copy(src.at[:, pl.ds(col * D, D)], stage.at[slot], sems.at[sem])

    cx = [pltpu.make_async_copy(x_hbm.at[:, pl.ds(c * 128, 128)], xio.at[c], sems.at[9 + c]) for c in range(8)]
    cps = [wcopy(awqkv_hbm, c, i, i + 1) for i, c in enumerate((1, 2, 0))]
    cwo = [pltpu.make_async_copy(awo_hbm.at[pl.ds(g * 256, 256), pl.ds(c * 128, 128)], wos.at[c * 4 + g], sems.at[4])
           for c in range(8) for g in range(4)]
    cps.append(None)
    srcs = [(bwqkv_hbm, 1), (bwqkv_hbm, 2), (bwqkv_hbm, 0), (bwo_hbm, 0)]
    cps += [wcopy(s, c, i + 3, i + 5) for i, (s, c) in enumerate(srcs)]
    for c in cps[:1] + cx + cps[1:2]:
        c.start()

    xu = xio.bitcast(U32)

    def in_body(c, _):
        pltpu.make_async_copy(xio.at[0], xio.at[0], sems.at[9 + c]).wait()

        @pl.when(c == 3)
        def _():
            for cp in [cps[2]] + cwo:
                cp.start()
        rows = pl.ds(pl.multiple_of(c * 128, 128), 128)
        for m in range(8):
            lo, hi = _unpack(xu[c, pl.ds(m, 128, stride=8), :].T)
            xt[rows, m * 128:(m + 1) * 128] = lo
            xt[rows, (8 + m) * 128:(9 + m) * 128] = hi
    def ln_tile(src, dst):
        for i in range(2):
            cs = [pl.ds(pl.multiple_of(jnp.int32(src) * NT + j * 128, 128), 128) for j in (i, i + 2)]
            st = []
            for c in cs:
                acc = xt[0:16, c]
                for r in range(16, D, 16):
                    acc = acc + xt[r:r + 16, c]
                m = jnp.sum(acc, axis=0, keepdims=True) * (1.0 / D)
                m = jnp.broadcast_to(m, (16, 128))
                acc = None
                for r in range(0, D, 16):
                    e = xt[r:r + 16, c] - m
                    acc = e * e if acc is None else acc + e * e
                v = jnp.sum(acc, axis=0, keepdims=True) * (1.0 / D)
                st.append((m, jnp.broadcast_to(lax.rsqrt(v + 1e-5), (16, 128))))
            for r in range(0, 512, 16):
                quads = [(xt[r0 + r:r0 + r + 16, cs[j]] - st[j][0]) * st[j][1] for r0 in (0, 512) for j in (0, 1)]
                for n, v in enumerate(_rhs7(*quads)):
                    xs[dst, n, r:r + 16, i * 128:(i + 1) * 128] = v

    def load_x():
        with jax.named_scope("loop_in"):
            lax.fori_loop(0, 8, in_body, None)
        for cp in cps[4:]:
            cp.start()
        with jax.named_scope("loop_ln"):
            lax.fori_loop(0, T, lambda t, c: ln_tile(t, t), None)

    def emit(mat, mc, r0, c0, *quads):
        for i, v in enumerate(_lhs7(*quads)):
            ws[mat * 2 + mc, i, r0:r0 + v.shape[0], c0:c0 + v.shape[1]] = v

    def prep_a(part, mc):
        tu = tb.bitcast(U32)
        for c in range(4):
            quads = []
            for j, (g, cc) in enumerate(((mc, c), (mc, c + 4), (mc + 2, c), (mc + 2, c + 4))):
                tb[j] = stage[part, cc * 128:(cc + 1) * 128, pl.ds(pl.multiple_of(g * 256, 256), 256)].T
                rows = []
                for e in range(16):
                    rows += list(_unpack(tu[j, pl.ds(e, 8, stride=16), :]))
                quads.append(jnp.concatenate(rows, 0))
            emit(part, mc, 0, c * 128, *quads)

    def prep_rest(mc):
        prep_a(2, mc)
        su = wos.bitcast(U32)
        for c in range(2):
            for gk in range(2):
                quads = []
                for cc, g in ((2 * mc + c, gk), (2 * mc + c, gk + 2), (2 * mc + c + 4, gk), (2 * mc + c + 4, gk + 2)):
                    rows = []
                    for e in range(16):
                        rows += list(_unpack(su[cc * 4 + g, pl.ds(e, 8, stride=16), :]))
                    quads.append(jnp.concatenate(rows, 0).T)
                emit(3, mc, c * 128, gk * 256, *quads)

    def prep_plain(slot, mat, mc):
        for c in range(4):
            quads = [stage[slot, cc * 128:(cc + 1) * 128, pl.ds(pl.multiple_of(g * 256, 256), 256)].T.astype(F32)
                     for g, cc in ((mc, c), (mc, c + 4), (mc + 2, c), (mc + 2, c + 4))]
            emit(mat, mc, 0, c * 128, *quads)

    def prep_fold(part, mc):
        zero = jnp.zeros((32, 32), F32)
        for gg in range(2):
            r = []
            for g in (mc, mc + 2):
                bd = jnp.concatenate(
                    [jnp.concatenate([bwphi_ref[8 * g + 4 * gg + i].astype(F32) if i == j else zero
                                      for j in range(4)], 1) for i in range(4)], 0).T.astype(BF16)
                wt = stage[3 + part, :, pl.ds(pl.multiple_of(g * 256 + gg * 128, 128), 128)].T
                r.append(_dot(bd, wt) * LOG2E)
            emit(4 + part, mc, gg * 128, 0, r[0][:, :512], r[0][:, 512:], r[1][:, :512], r[1][:, 512:])

    def first(part):
        cps[part].wait()
        with jax.named_scope("loop_pa"):
            lax.fori_loop(0, 2, lambda g, c: prep_a(part, g), None)
    first(0)
    load_x()
    first(1)
    for c in [cps[2]] + cwo:
        c.wait()
    with jax.named_scope("loop_pr"):
        lax.fori_loop(0, 2, lambda g, c: prep_rest(g), None)

    def sdot(mat, mc, rhs, k0=0, k1=512):
        p = [_dot(ws[mat * 2 + mc, i, :, k0:k1], rhs(i)[k0:k1, :]) for i in range(7)]
        return (jnp.concatenate([p[0] + p[3] - p[4] + p[6], p[2] + p[4]], 1),
                jnp.concatenate([p[1] + p[3], p[0] - p[1] + p[2] + p[5]], 1))

    def xdot(mat, mc, t):
        return sdot(mat, mc, lambda i: xs.at[t, i])

    def wo_part(mat, half):
        p = [sdot(mat, mc, lambda i: os_.at[i], *((0, 512) if mat == 7 else (half * 256, half * 256 + 256))) for mc in range(2)]
        return jnp.concatenate([p[0][0], p[1][0], p[0][1], p[1][1]], 0)

    def finish(mat, t, cols, part):
        xt[:, cols] = part + wo_part(mat, 1)


    def emit_o(half, r0, c0, *quads, dst=os_):
        for i, v in enumerate(_rhs7(*quads)):
            dst[i, half * 256 + r0:half * 256 + r0 + v.shape[0], c0:c0 + v.shape[1]] = v

    def layer_a(it):
        def kv_body(t, _):
            cols = pl.ds(pl.multiple_of(jnp.int32(t) * NT, NT), NT)
            base = t * NB + 8 * (t * NB // 8)
            for part, dst in ((0, k2), (1, v2)):
                for mc in range(2):
                    for g, r in zip((mc, mc + 2), xdot(part, mc, t)):
                        for i in range(NB):
                            blk = r[:, i * 128:(i + 1) * 128]
                            dst[base + i + 8, g * 256:(g + 1) * 256] = blk
                            dst[base + i, g * 256:(g + 1) * 256] = pltpu.roll(blk, 1, 1)
            return 0
        with jax.named_scope("loop137"):
            lax.fori_loop(0, T, kv_body, 0)

        @pl.when(it == 0)
        def _():
            for c in cps[4:]:
                c.wait()

            def prep_b(mc, _):
                prep_fold(0, mc)
                prep_fold(2, mc)
                prep_plain(4, 5, mc)
                prep_plain(6, 7, mc)
            lax.fori_loop(0, 2, prep_b, None)

        def q_body(t, _):
            cols = pl.ds(pl.multiple_of(jnp.int32(t) * NT, NT), NT)
            base = t * NB + 8 * (t * NB // 8)
            m0 = t * NB % 8
            lane0 = lax.broadcasted_iota(jnp.int32, (8, 128), 1) == 0
            qs = [xdot(2, 0, t), xdot(2, 1, t)]
            ln_tile(jnp.maximum(t - 1, 0), jnp.where(t == 0, T, t - 1))
            for g in (0, 2, 1, 3):
                q = qs[g % 2][g // 2]
                if g == 1:
                    part = xt[:, cols] + wo_part(3, 0)
                if g < 2:
                    outs = []
                for i in range(NB):
                    lg = []
                    for w in range(W):
                        acc = None
                        for d in range(DH):
                            pr = (q[d * 8:(d + 1) * 8, i * 128:(i + 1) * 128]
                                  * k2[base + i + 8 - w, g * 256 + d * 8: g * 256 + (d + 1) * 8, :])
                            acc = pr if acc is None else acc + pr
                        acc = acc * (DH ** -0.5 * LOG2E)
                        if w > i:
                            acc = jnp.where(jnp.logical_and(lane0, m0 + i < w), -1e9 * LOG2E, acc)
                        lg.append(acc)
                    mx = lg[0]
                    for w in range(1, W):
                        mx = jnp.maximum(mx, lg[w])
                    es = [jnp.exp2(l - mx) for l in lg]
                    tot = es[0]
                    for w in range(1, W):
                        tot = tot + es[w]
                    inv = _rcp(tot)
                    ps = [e * inv for e in es]
                    rows = []
                    for d in range(DH):
                        acc = None
                        for w in range(W):
                            pr = ps[w] * v2[base + i + 8 - w, g * 256 + d * 8: g * 256 + (d + 1) * 8, :]
                            acc = pr if acc is None else acc + pr
                        rows.append(acc)
                    outs.append(jnp.concatenate(rows, 0))
                if g >= 2:
                    for i in range(2):
                        emit_o(g - 2, 0, i * 128, outs[i], outs[i + 2], outs[4 + i], outs[6 + i])
            finish(3, t, cols, part)
            return 0
        with jax.named_scope("loop178"):
            lax.fori_loop(0, T, q_body, 0)

    def layer_b():
        kvb[...] = jnp.zeros(kvb.shape, F32)

        def kv_body(t, _):
            cols = pl.ds(pl.multiple_of(jnp.int32(t) * NT, NT), NT)
            ones = jnp.ones((16, NT), BF16)
            ks = [xdot(4, mc, t) for mc in range(2)]
            vs = [xdot(5, mc, t) for mc in range(2)]
            if isinstance(t, int) and t == 0:
                ln_tile(T - 1, T - 1)
            for g in (0, 2, 1, 3):
                k = ks[g % 2][g // 2]
                v = vs[g % 2][g // 2].astype(BF16)
                for i in range(4):
                    phi = jnp.concatenate([_dual_softmax(k[i * 64:i * 64 + 32]),
                                           _dual_softmax(k[i * 64 + 32:i * 64 + 64])], 0)
                    lhs = jnp.concatenate([v[i * 64:(i + 1) * 64], ones], 0)
                    kvb[g * 4 + i] += _dot_nt(lhs, phi)
            return 0
        with jax.named_scope("loop195"):
            kv_body(0, 0)
            lax.fori_loop(1, T, kv_body, 0)
        r = lax.broadcasted_iota(jnp.int32, (80, 128), 0)
        c = lax.broadcasted_iota(jnp.int32, (80, 128), 1)
        keep = jnp.where(r < 64, r // 32, (r - 64) // 8) == c // 64
        for i in range(16):
            kvb[i] = jnp.where(keep, kvb[i], 0.0)

        def chunk(t, mc, qq):
            for i in range(4):
                outs = []
                for j in range(2):
                    q = qq[j]
                    phi = jnp.concatenate([_dual_softmax(q[i * 64:i * 64 + 32]),
                                           _dual_softmax(q[i * 64 + 32:i * 64 + 64])], 0)
                    nd = _dot(kvb[(mc + 2 * j) * 4 + i].astype(BF16), phi)
                    rows = []
                    for hh in range(2):
                        inv = _rcp(nd[64 + hh * 8:72 + hh * 8] + 1e-6)
                        rows += [nd[hh * 32 + r * 8: hh * 32 + (r + 1) * 8] * inv for r in range(4)]
                    outs.append(jnp.concatenate(rows, 0))
                emit_o(mc, i * 64, 0, outs[0][:, :256], outs[0][:, 256:], outs[1][:, :256], outs[1][:, 256:],
                       dst=(os_, os2)[t % 2])

        with jax.named_scope("loop217"):
            q0 = xdot(6, 0, 0)
            q1 = xdot(6, 1, 0)
            chunk(0, 0, q0)
            for t in range(T):
                if t + 1 < T:
                    q0 = xdot(6, 0, t + 1)
                chunk(t, 1, q1)
                if t + 1 < T:
                    q1 = xdot(6, 1, t + 1)
                src = (os_, os2)[t % 2]
                p = [sdot(7, mc, lambda i: src.at[i]) for mc in range(2)]
                cols = slice(t * NT, (t + 1) * NT)
                x = xt[:, cols] + jnp.concatenate([p[0][0], p[1][0], p[0][1], p[1][1]], 0)
                xt[:, cols] = x
                ln_tile(t, t)
                if t + 1 < T:
                    chunk(t + 1, 0, q0)

    def pair(it, c):
        layer_a(it)
        layer_b()
        return c
    lax.fori_loop(0, 2, pair, 0)

    co = [pltpu.make_async_copy(xio.at[c], o_hbm.at[:, pl.ds(c * 128, 128)], sems.at[0]) for c in range(8)]

    def out_body(c, _):
        rows = pl.ds(pl.multiple_of(c * 128, 128), 128)
        for m in range(8):
            lo, hi = [pltpu.bitcast(xt[rows, b * 128:(b + 1) * 128].astype(BF16).astype(F32), U32)
                      for b in (m, 8 + m)]
            xu[c, pl.ds(m, 128, stride=8), :] = ((lo >> 16) | hi).T
        pltpu.make_async_copy(xio.at[c], o_hbm.at[:, pl.ds(pl.multiple_of(c * 128, 128), 128)], sems.at[0]).start()
    with jax.named_scope("loop_out"):
        lax.fori_loop(0, 8, out_body, None)
    for c in co:
        c.wait()


@jax.jit
def pallas_interleave_layers__sliding_local_dilated__linear_kernel_hedgehog__prompt_kernel(
    A_x, A_wqkv, A_wo, B_x, B_wqkv, B_w_phi, B_wo,
):
    hbm = pl.BlockSpec(memory_space=pl.ANY)
    out = pl.pallas_call(
        _kernel,
        out_shape=jax.ShapeDtypeStruct((S, D), BF16),
        in_specs=[hbm, hbm, hbm, hbm, pl.BlockSpec(memory_space=pltpu.VMEM), hbm],
        out_specs=hbm,
        scratch_shapes=[
            pltpu.VMEM((8, S, 128), BF16),
            pltpu.VMEM((7, D, D), BF16),
            pltpu.VMEM((32, 256, 128), BF16),
            pltpu.VMEM((4, 256, 128), BF16),
            pltpu.VMEM((16, 7, 256, 512), BF16),
            pltpu.VMEM((D, S), F32),
            pltpu.VMEM((T + 1, 7, 512, 256), BF16),
            pltpu.VMEM((32, D, 128), F32),
            pltpu.VMEM((32, D, 128), F32),
            pltpu.VMEM((7, 512, 256), BF16),
            pltpu.VMEM((7, 512, 256), BF16),
            pltpu.VMEM((16, 80, 128), F32),
            pltpu.SemaphoreType.DMA((17,)),
        ],
        compiler_params=pltpu.CompilerParams(vmem_limit_bytes=126 * 1024 * 1024),
    )(A_x.reshape(S, D), A_wqkv, A_wo, B_wqkv, B_w_phi, B_wo)
    return out.reshape(1, S, D)
```

```python
import jax
import jax.numpy as jnp
from jax import lax
import jax.experimental.pallas as pl
import jax.experimental.pallas.tpu as pltpu

S, D, H, DH, W = 2048, 1024, 32, 32, 8
NT = 512
NB = NT // 128
T = S // NT
LOG2E = 1.4426950408889634
F32, BF16, U32 = jnp.float32, jnp.bfloat16, jnp.uint32


def _dot(a, b):
    return jnp.dot(a, b, preferred_element_type=F32)


def _dot_nt(a, b):
    return lax.dot_general(a, b, (((1,), (1,)), ((), ())), preferred_element_type=F32)


def _rcp(x):
    return pl.reciprocal(x, approx=True)


def _unpack(u):
    lo = pltpu.bitcast(u << 16, F32)
    hi = pltpu.bitcast(u & jnp.uint32(0xFFFF0000), F32)
    return lo, hi


def _rhs7(b11, b12, b21, b22):
    return [v.astype(BF16) for v in (b11 + b22, b11, b12 - b22, b21 - b11, b22, b11 + b12, b21 + b22)]


def _lhs7(a11, a12, a21, a22):
    return [v.astype(BF16) for v in (a11 + a22, a21 + a22, a11, a22, a11 + a12, a21 - a11, a12 - a22)]


def _dual_softmax(p):
    return jnp.concatenate([_ds(p[:, i:i + 128]) for i in range(0, p.shape[1], 128)], 1)


def _ds(p):
    ep = jnp.exp2(p - jnp.max(p, axis=0, keepdims=True))
    en = jnp.exp2(jnp.min(p, axis=0, keepdims=True) - p)
    ep = ep * _rcp(jnp.sum(ep, axis=0, keepdims=True))
    en = en * _rcp(jnp.sum(en, axis=0, keepdims=True))
    return jnp.concatenate([ep, en], axis=0).astype(BF16)


def _kernel(x_hbm, awqkv_hbm, awo_hbm, bwqkv_hbm, bwphi_ref, bwo_hbm, o_hbm,
            xio, stage, wos, tb, ws, xt, xs, k2, v2, os_, os2, kvb, sems):
    def wcopy(src, col, slot, sem):
        return pltpu.make_async_copy(src.at[:, pl.ds(col * D, D)], stage.at[slot], sems.at[sem])

    cx = [pltpu.make_async_copy(x_hbm.at[:, pl.ds(c * 128, 128)], xio.at[c], sems.at[9 + c]) for c in range(8)]
    cps = [wcopy(awqkv_hbm, c, i, i + 1) for i, c in enumerate((1, 2, 0))]
    cwo = [pltpu.make_async_copy(awo_hbm.at[pl.ds(g * 256, 256), pl.ds(c * 128, 128)], wos.at[c * 4 + g], sems.at[4])
           for c in range(8) for g in range(4)]
    cps.append(None)
    srcs = [(bwqkv_hbm, 1), (bwqkv_hbm, 2), (bwqkv_hbm, 0), (bwo_hbm, 0)]
    cps += [wcopy(s, c, i + 3, i + 5) for i, (s, c) in enumerate(srcs)]
    for c in cps[:1] + cx + cps[1:2]:
        c.start()

    xu = xio.bitcast(U32)

    def in_body(c, _):
        pltpu.make_async_copy(xio.at[0], xio.at[0], sems.at[9 + c]).wait()

        @pl.when(c == 3)
        def _():
            for cp in [cps[2]] + cwo:
                cp.start()
        rows = pl.ds(pl.multiple_of(c * 128, 128), 128)
        for m in range(8):
            lo, hi = _unpack(xu[c, pl.ds(m, 128, stride=8), :].T)
            xt[rows, m * 128:(m + 1) * 128] = lo
            xt[rows, (8 + m) * 128:(9 + m) * 128] = hi
    def ln_tile(src, dst):
        for i in range(2):
            cs = [pl.ds(pl.multiple_of(jnp.int32(src) * NT + j * 128, 128), 128) for j in (i, i + 2)]
            st = []
            for c in cs:
                acc = xt[0:16, c]
                for r in range(16, D, 16):
                    acc = acc + xt[r:r + 16, c]
                m = jnp.sum(acc, axis=0, keepdims=True) * (1.0 / D)
                m = jnp.broadcast_to(m, (16, 128))
                acc = None
                for r in range(0, D, 16):
                    e = xt[r:r + 16, c] - m
                    acc = e * e if acc is None else acc + e * e
                v = jnp.sum(acc, axis=0, keepdims=True) * (1.0 / D)
                st.append((m, jnp.broadcast_to(lax.rsqrt(v + 1e-5), (16, 128))))
            for r in range(0, 512, 16):
                quads = [(xt[r0 + r:r0 + r + 16, cs[j]] - st[j][0]) * st[j][1] for r0 in (0, 512) for j in (0, 1)]
                for n, v in enumerate(_rhs7(*quads)):
                    xs[dst, n, r:r + 16, i * 128:(i + 1) * 128] = v

    def load_x():
        with jax.named_scope("loop_in"):
            lax.fori_loop(0, 8, in_body, None)
        for cp in cps[4:]:
            cp.start()
        with jax.named_scope("loop_ln"):
            lax.fori_loop(0, T - 1, lambda t, c: ln_tile(t, t), None)

    def emit(mat, mc, r0, c0, *quads):
        for i, v in enumerate(_lhs7(*quads)):
            ws[mat * 2 + mc, i, r0:r0 + v.shape[0], c0:c0 + v.shape[1]] = v

    def prep_a(part, mc):
        tu = tb.bitcast(U32)
        for c in range(4):
            quads = []
            for j, (g, cc) in enumerate(((mc, c), (mc, c + 4), (mc + 2, c), (mc + 2, c + 4))):
                tb[j] = stage[part, cc * 128:(cc + 1) * 128, pl.ds(pl.multiple_of(g * 256, 256), 256)].T
                rows = []
                for e in range(16):
                    rows += list(_unpack(tu[j, pl.ds(e, 8, stride=16), :]))
                quads.append(jnp.concatenate(rows, 0))
            emit(part, mc, 0, c * 128, *quads)

    def prep_rest(mc):
        prep_a(2, mc)
        su = wos.bitcast(U32)
        for c in range(2):
            for gk in range(2):
                quads = []
                for cc, g in ((2 * mc + c, gk), (2 * mc + c, gk + 2), (2 * mc + c + 4, gk), (2 * mc + c + 4, gk + 2)):
                    rows = []
                    for e in range(16):
                        rows += list(_unpack(su[cc * 4 + g, pl.ds(e, 8, stride=16), :]))
                    quads.append(jnp.concatenate(rows, 0).T)
                emit(3, mc, c * 128, gk * 256, *quads)

    def prep_plain(slot, mat, mc):
        for c in range(4):
            quads = [stage[slot, cc * 128:(cc + 1) * 128, pl.ds(pl.multiple_of(g * 256, 256), 256)].T.astype(F32)
                     for g, cc in ((mc, c), (mc, c + 4), (mc + 2, c), (mc + 2, c + 4))]
            emit(mat, mc, 0, c * 128, *quads)

    def prep_fold(part, mc):
        zero = jnp.zeros((32, 32), F32)
        for gg in range(2):
            r = []
            for g in (mc, mc + 2):
                bd = jnp.concatenate(
                    [jnp.concatenate([bwphi_ref[8 * g + 4 * gg + i].astype(F32) if i == j else zero
                                      for j in range(4)], 1) for i in range(4)], 0).T.astype(BF16)
                wt = stage[3 + part, :, pl.ds(pl.multiple_of(g * 256 + gg * 128, 128), 128)].T
                r.append(_dot(bd, wt) * LOG2E)
            emit(4 + part, mc, gg * 128, 0, r[0][:, :512], r[0][:, 512:], r[1][:, :512], r[1][:, 512:])

    def first(part):
        cps[part].wait()
        with jax.named_scope("loop_pa"):
            lax.fori_loop(0, 2, lambda g, c: prep_a(part, g), None)
    first(0)
    load_x()
    first(1)
    for c in [cps[2]] + cwo:
        c.wait()
    with jax.named_scope("loop_pr"):
        lax.fori_loop(0, 2, lambda g, c: prep_rest(g), None)

    def sdot(mat, mc, rhs, k0=0, k1=512):
        p = [_dot(ws[mat * 2 + mc, i, :, k0:k1], rhs(i)[k0:k1, :]) for i in range(7)]
        return (jnp.concatenate([p[0] + p[3] - p[4] + p[6], p[2] + p[4]], 1),
                jnp.concatenate([p[1] + p[3], p[0] - p[1] + p[2] + p[5]], 1))

    def xdot(mat, mc, t):
        return sdot(mat, mc, lambda i: xs.at[t, i])

    def wo_part(mat, half):
        p = [sdot(mat, mc, lambda i: os_.at[i], *((0, 512) if mat == 7 else (half * 256, half * 256 + 256))) for mc in range(2)]
        return jnp.concatenate([p[0][0], p[1][0], p[0][1], p[1][1]], 0)

    def finish(mat, t, cols, part):
        xt[:, cols] = part + wo_part(mat, 1)


    def emit_o(half, r0, c0, *quads, dst=os_):
        for i, v in enumerate(_rhs7(*quads)):
            dst[i, half * 256 + r0:half * 256 + r0 + v.shape[0], c0:c0 + v.shape[1]] = v

    def layer_a(it):
        def kv_body(t, _):
            cols = pl.ds(pl.multiple_of(jnp.int32(t) * NT, NT), NT)
            base = t * NB + 8 * (t * NB // 8)
            for part, dst in ((0, k2), (1, v2)):
                for mc in range(2):
                    for g, r in zip((mc, mc + 2), xdot(part, mc, t)):
                        for i in range(NB):
                            blk = r[:, i * 128:(i + 1) * 128]
                            dst[base + i + 8, g * 256:(g + 1) * 256] = blk
                            dst[base + i, g * 256:(g + 1) * 256] = pltpu.roll(blk, 1, 1)
            return 0
        with jax.named_scope("loop137"):
            ln_tile(T - 1, T - 1)
            kv_body(0, 0)
            lax.fori_loop(1, T, kv_body, 0)

        @pl.when(it == 0)
        def _():
            for c in cps[4:]:
                c.wait()

            def prep_b(mc, _):
                prep_fold(0, mc)
                prep_fold(2, mc)
                prep_plain(4, 5, mc)
                prep_plain(6, 7, mc)
            lax.fori_loop(0, 2, prep_b, None)

        def q_body(t, _):
            cols = pl.ds(pl.multiple_of(jnp.int32(t) * NT, NT), NT)
            base = t * NB + 8 * (t * NB // 8)
            m0 = t * NB % 8
            lane0 = lax.broadcasted_iota(jnp.int32, (8, 128), 1) == 0
            qs = [xdot(2, 0, t), xdot(2, 1, t)]
            ln_tile(jnp.maximum(t - 1, 0), jnp.where(t == 0, T, t - 1))
            for g in (0, 2, 1, 3):
                q = qs[g % 2][g // 2]
                if g == 1:
                    part = xt[:, cols] + wo_part(3, 0)
                if g < 2:
                    outs = []
                for i in range(NB):
                    lg = []
                    for w in range(W):
                        acc = None
                        for d in range(DH):
                            pr = (q[d * 8:(d + 1) * 8, i * 128:(i + 1) * 128]
                                  * k2[base + i + 8 - w, g * 256 + d * 8: g * 256 + (d + 1) * 8, :])
                            acc = pr if acc is None else acc + pr
                        acc = acc * (DH ** -0.5 * LOG2E)
                        if w > i:
                            acc = jnp.where(jnp.logical_and(lane0, m0 + i < w), -1e9 * LOG2E, acc)
                        lg.append(acc)
                    mx = lg[0]
                    for w in range(1, W):
                        mx = jnp.maximum(mx, lg[w])
                    es = [jnp.exp2(l - mx) for l in lg]
                    tot = es[0]
                    for w in range(1, W):
                        tot = tot + es[w]
                    inv = _rcp(tot)
                    ps = [e * inv for e in es]
                    rows = []
                    for d in range(DH):
                        acc = None
                        for w in range(W):
                            pr = ps[w] * v2[base + i + 8 - w, g * 256 + d * 8: g * 256 + (d + 1) * 8, :]
                            acc = pr if acc is None else acc + pr
                        rows.append(acc)
                    outs.append(jnp.concatenate(rows, 0))
                if g >= 2:
                    for i in range(2):
                        emit_o(g - 2, 0, i * 128, outs[i], outs[i + 2], outs[4 + i], outs[6 + i])
            finish(3, t, cols, part)
            return 0
        with jax.named_scope("loop178"):
            lax.fori_loop(0, T, q_body, 0)

    def layer_b():
        kvb[...] = jnp.zeros(kvb.shape, F32)

        def kv_body(t, _):
            cols = pl.ds(pl.multiple_of(jnp.int32(t) * NT, NT), NT)
            ones = jnp.ones((16, NT), BF16)
            ks = [xdot(4, mc, t) for mc in range(2)]
            vs = [xdot(5, mc, t) for mc in range(2)]
            if isinstance(t, int) and t == 0:
                ln_tile(T - 1, T - 1)
            for g in (0, 2, 1, 3):
                k = ks[g % 2][g // 2]
                v = vs[g % 2][g // 2].astype(BF16)
                for i in range(4):
                    phi = jnp.concatenate([_dual_softmax(k[i * 64:i * 64 + 32]),
                                           _dual_softmax(k[i * 64 + 32:i * 64 + 64])], 0)
                    lhs = jnp.concatenate([v[i * 64:(i + 1) * 64], ones], 0)
                    kvb[g * 4 + i] += _dot_nt(lhs, phi)
            return 0
        with jax.named_scope("loop195"):
            kv_body(0, 0)
            lax.fori_loop(1, T, kv_body, 0)
        r = lax.broadcasted_iota(jnp.int32, (80, 128), 0)
        c = lax.broadcasted_iota(jnp.int32, (80, 128), 1)
        keep = jnp.where(r < 64, r // 32, (r - 64) // 8) == c // 64
        for i in range(16):
            kvb[i] = jnp.where(keep, kvb[i], 0.0)

        def chunk(t, mc, qq):
            for i in range(4):
                outs = []
                for j in range(2):
                    q = qq[j]
                    phi = jnp.concatenate([_dual_softmax(q[i * 64:i * 64 + 32]),
                                           _dual_softmax(q[i * 64 + 32:i * 64 + 64])], 0)
                    nd = _dot(kvb[(mc + 2 * j) * 4 + i].astype(BF16), phi)
                    rows = []
                    for hh in range(2):
                        inv = _rcp(nd[64 + hh * 8:72 + hh * 8] + 1e-6)
                        rows += [nd[hh * 32 + r * 8: hh * 32 + (r + 1) * 8] * inv for r in range(4)]
                    outs.append(jnp.concatenate(rows, 0))
                emit_o(mc, i * 64, 0, outs[0][:, :256], outs[0][:, 256:], outs[1][:, :256], outs[1][:, 256:],
                       dst=(os_, os2)[t % 2])

        with jax.named_scope("loop217"):
            q0 = xdot(6, 0, 0)
            q1 = xdot(6, 1, 0)
            chunk(0, 0, q0)
            for t in range(T):
                if t + 1 < T:
                    q0 = xdot(6, 0, t + 1)
                chunk(t, 1, q1)
                if t + 1 < T:
                    q1 = xdot(6, 1, t + 1)
                if t:
                    ln_tile(t - 1, t - 1)
                src = (os_, os2)[t % 2]
                p = [sdot(7, mc, lambda i: src.at[i]) for mc in range(2)]
                cols = slice(t * NT, (t + 1) * NT)
                x = xt[:, cols] + jnp.concatenate([p[0][0], p[1][0], p[0][1], p[1][1]], 0)
                xt[:, cols] = x
                if t + 1 < T:
                    chunk(t + 1, 0, q0)

    def pair(it, c):
        layer_a(it)
        layer_b()
        return c
    lax.fori_loop(0, 2, pair, 0)

    co = [pltpu.make_async_copy(xio.at[c], o_hbm.at[:, pl.ds(c * 128, 128)], sems.at[0]) for c in range(8)]

    def out_body(c, _):
        rows = pl.ds(pl.multiple_of(c * 128, 128), 128)
        for m in range(8):
            lo, hi = [pltpu.bitcast(xt[rows, b * 128:(b + 1) * 128].astype(BF16).astype(F32), U32)
                      for b in (m, 8 + m)]
            xu[c, pl.ds(m, 128, stride=8), :] = ((lo >> 16) | hi).T
        pltpu.make_async_copy(xio.at[c], o_hbm.at[:, pl.ds(pl.multiple_of(c * 128, 128), 128)], sems.at[0]).start()
    with jax.named_scope("loop_out"):
        lax.fori_loop(0, 8, out_body, None)
    for c in co:
        c.wait()


@jax.jit
def pallas_interleave_layers__sliding_local_dilated__linear_kernel_hedgehog__prompt_kernel(
    A_x, A_wqkv, A_wo, B_x, B_wqkv, B_w_phi, B_wo,
):
    hbm = pl.BlockSpec(memory_space=pl.ANY)
    out = pl.pallas_call(
        _kernel,
        out_shape=jax.ShapeDtypeStruct((S, D), BF16),
        in_specs=[hbm, hbm, hbm, hbm, pl.BlockSpec(memory_space=pltpu.VMEM), hbm],
        out_specs=hbm,
        scratch_shapes=[
            pltpu.VMEM((8, S, 128), BF16),
            pltpu.VMEM((7, D, D), BF16),
            pltpu.VMEM((32, 256, 128), BF16),
            pltpu.VMEM((4, 256, 128), BF16),
            pltpu.VMEM((16, 7, 256, 512), BF16),
            pltpu.VMEM((D, S), F32),
            pltpu.VMEM((T + 1, 7, 512, 256), BF16),
            pltpu.VMEM((32, D, 128), F32),
            pltpu.VMEM((32, D, 128), F32),
            pltpu.VMEM((7, 512, 256), BF16),
            pltpu.VMEM((7, 512, 256), BF16),
            pltpu.VMEM((16, 80, 128), F32),
            pltpu.SemaphoreType.DMA((17,)),
        ],
        compiler_params=pltpu.CompilerParams(vmem_limit_bytes=126 * 1024 * 1024),
    )(A_x.reshape(S, D), A_wqkv, A_wo, B_wqkv, B_w_phi, B_wo)
    return out.reshape(1, S, D)
```
